```python
import os as _os
_os.environ.setdefault('JAX_PLATFORMS', 'cpu')
import jax
import jax.numpy as jnp

def _softmax(x, axis=-1):
    return jax.nn.softmax(x, axis=axis)

def _gelu(x):
    return jax.nn.gelu(x, approximate=True)

def _silu(x):
    return jax.nn.silu(x)

def _sigmoid(x):
    return jax.nn.sigmoid(x)

def _layernorm(x, axis=-1, eps=1e-05):
    m = jnp.mean(x, axis=axis, keepdims=True)
    v = jnp.var(x, axis=axis, keepdims=True)
    return (x - m) / jnp.sqrt(v + eps)

def _scatter_add(tgt, idx, src, axis=0):
    return tgt.at[idx].add(src)

def _segment_sum(src, seg, n):
    return jax.ops.segment_sum(src, seg, n)

class _Rng:

    def __init__(self, key):
        self._k = key

    def _next(self):
        self._k, sub = jax.random.split(self._k)
        return sub

    def normal(self, shape):
        return jax.random.normal(self._next(), shape, dtype=jnp.bfloat16)

    def randint(self, lo, hi, shape):
        return jax.random.randint(self._next(), shape, lo, hi, dtype=jnp.int32)

    def uniform(self, shape, lo=0.0, hi=1.0):
        return jax.random.uniform(self._next(), shape, jnp.bfloat16, lo, hi)

    def permutation(self, n):
        return jax.random.permutation(self._next(), n)
kernel_name = 'adaLN_cond__memory_aug_recurrent_mem_tr__moe_arch_mod__prompt'

def setup_inputs():
    _rng = _Rng(jax.random.key(int.from_bytes(__import__("os").urandom(4), "little")))
    _w = lambda a: (lambda t: t.astype(jnp.bfloat16) if jnp.issubdtype(t.dtype, jnp.floating) else t)(jnp.asarray(a))

    def _A_setup():
        B, S, Dm = (1, 2048, 448)
        H, Dh = (16, 256)
        M, seg = (8, 32)
        seg = min(seg, S)
        S = S // seg * seg
        return {'x': _w((lambda *s: _rng.normal(s) * 0.05)(B, S, Dm)), 'mem0': _w((lambda *s: _rng.normal(s) * 0.4)(B, M, Dm)), 'Wq': _w((lambda *s: _rng.normal(s) * 1.6)(Dm, H, Dh) * Dm ** (-0.5)), 'Wk': _w((lambda *s: _rng.normal(s) * 1.6)(Dm, H, Dh) * Dm ** (-0.5)), 'Wv': _w((lambda *s: _rng.normal(s) * 0.4)(Dm, H, Dh) * Dm ** (-0.5)), 'Wo': _w((lambda *s: _rng.normal(s) * 0.4)(H, Dh, Dm) * (H * Dh) ** (-0.5)), 'seg_len': seg}
    _A_in = _A_setup()

    def _B_setup():
        B, S, D, F, C = (1, 2048, 448, 1792, 1)
        return {'x': _w((lambda *s: _rng.normal(s) * 0.05)(B, S, D)), 'w_r': _w((lambda *s: _rng.normal(s) * 0.05)(D)), 'w_gate': _w((lambda *s: _rng.normal(s) * 0.05)(D, F)), 'w_up': _w((lambda *s: _rng.normal(s) * 0.05)(D, F)), 'w_down': _w((lambda *s: _rng.normal(s) * 0.05)(F, D))}
    _B_in = _B_setup()
    return {'A_x': _A_in['x'], 'A_mem0': _A_in['mem0'], 'A_Wq': _A_in['Wq'], 'A_Wk': _A_in['Wk'], 'A_Wv': _A_in['Wv'], 'A_Wo': _A_in['Wo'], 'A_seg_len': _A_in['seg_len'], 'B_x': _B_in['x'], 'B_w_r': _B_in['w_r'], 'B_w_gate': _B_in['w_gate'], 'B_w_up': _B_in['w_up'], 'B_w_down': _B_in['w_down'], 'c': _w((lambda *s: _rng.normal(s) * 0.05)(1, 448) * 8.0), 'w_mod': _w((lambda *s: _rng.normal(s) * 0.05)(448, 6 * 448) * 448 ** (-0.5) * 8.0)}

def reference(A_x, A_mem0, A_Wq, A_Wk, A_Wv, A_Wo, A_seg_len, B_x, B_w_r, B_w_gate, B_w_up, B_w_down, c, w_mod):

    def _A_ref(x, mem0, Wq, Wk, Wv, Wo, seg_len):
        B, S, Dm = x.shape
        H, Dh = (Wq.shape[1], Wq.shape[2])
        M = mem0.shape[1]
        scale = Dh ** (-0.5)
        n_seg = S // seg_len
        L = M + seg_len
        idx = jnp.arange(L)
        mask = (idx[:, None] < M) | (idx[:, None] >= idx[None, :])
        mem = mem0
        outs = []
        for s in range(n_seg):
            xs = x[:, s * seg_len:(s + 1) * seg_len, :].copy()
            h = jnp.concatenate([mem, xs], axis=1)
            q = jnp.einsum('btd,dhe->bhte', h, Wq)
            k = jnp.einsum('btd,dhe->bhte', h, Wk)
            v = jnp.einsum('btd,dhe->bhte', h, Wv)
            scores = jnp.einsum('bhqe,bhke->bhqk', q, k) * scale
            scores = jnp.where(mask[None, None], scores, -1000000000.0)
            p = _softmax(scores, axis=-1)
            o = jnp.einsum('bhqk,bhke->bhqe', p, v)
            o = jnp.einsum('bhte,hed->btd', o, Wo)
            mem = o[:, :M, :].copy()
            outs.append(o[:, M:, :])
        return jnp.concatenate(outs, axis=1)

    def _B_ref(x, w_r, w_gate, w_up, w_down):
        B, S, D = x.shape
        C = 1
        r = x @ w_r
        idx = jnp.argsort(-r, axis=-1)[:, :C]
        idx_e = jnp.repeat(idx.reshape(B, C, 1), D, axis=2)
        x_sel = jnp.take_along_axis(x, idx_e, axis=1)
        g = _silu(x_sel @ w_gate)
        u = x_sel @ w_up
        y = g * u @ w_down
        r_sel = _sigmoid(jnp.take_along_axis(r, idx, axis=1))
        y = y * r_sel.reshape(B, C, 1)
        b_off = (jnp.arange(B) * S).reshape(B, 1)
        flat_idx = (idx + b_off).reshape(B * C)
        zero = (x * 0.0).reshape(B * S, D)
        upd = _scatter_add(zero, flat_idx, y.reshape(B * C, D), axis=0)
        return x + upd.reshape(B, S, D)
    x = A_x
    mod = (_silu(c) @ w_mod).reshape(c.shape[0], 6, 1, -1)
    sa, ca, ga, sb, cb, gb = (mod[:, 0].copy(), mod[:, 1].copy(), mod[:, 2].copy(), mod[:, 3].copy(), mod[:, 4].copy(), mod[:, 5].copy())
    h = _layernorm(x, axis=-1) * (1 + ca) + sa
    x = x + ga * _A_ref(h, A_mem0, A_Wq, A_Wk, A_Wv, A_Wo, A_seg_len)
    h = _layernorm(x, axis=-1) * (1 + cb) + sb
    x = x + gb * _B_ref(h, B_w_r, B_w_gate, B_w_up, B_w_down)
    return x
```

```python
import functools

import jax
import jax.numpy as jnp
from jax import lax
from jax.experimental import pallas as pl
from jax.experimental.pallas import tpu as pltpu

F32 = jnp.float32
BF16 = jnp.bfloat16
U32 = jnp.uint32

S, D, H, E, M, SEG, FF = 2048, 448, 16, 256, 8, 32, 1792
DP = 512
NSEG = S // SEG
NG = S // 128
L = SEG + M
NW = H * D
NT = (((1,), (1,)), ((), ()))
EPS = 1e-5


def _dup(v):
    return jnp.concatenate([v, v[:, 384:448]], axis=1)


def _rowsum(v):
    t = v[:, 0:128] + v[:, 128:256] + v[:, 256:384] + 0.5 * v[:, 384:512]
    return jnp.sum(t, axis=1, keepdims=True)


def _layernorm(v):
    mu = _rowsum(v) * (1.0 / D)
    d = v - mu
    var = _rowsum(d * d) * (1.0 / D)
    return d * lax.rsqrt(var + EPS)


def _group8(v, op, lane):
    for d in (1, 2, 4):
        up = pltpu.roll(v, d, 1)
        dn = pltpu.roll(v, 128 - d, 1)
        v = op(v, jnp.where((lane & d) != 0, up, dn))
    return v


def _unpack(u):
    lo = pltpu.bitcast(u << 16, F32)
    hi = pltpu.bitcast(u & jnp.uint32(0xFFFF0000), F32)
    return lo, hi


def _kernel(xT_hbm, mem0_ref, wq_hbm, wk_hbm, wv_hbm, woT_hbm, wr_ref, wg_hbm, wu_hbm, wdT_hbm,
            c_ref, wmod_hbm, out_hbm,
            wq_v, wk_v, wv_v, wo_v, wmod_v, wg_v, wu_v, wd_v, xs_v, w_s, vec_s,
            x_s, o_s, h2_s, st_s, hbuf, obuf, sems, osems):
    def half(src, dst, t, k):
        return pltpu.make_async_copy(src.at[:, pl.ds(128 * t, 128)], dst.at[t], sems.at[k])

    cp_mod = pltpu.make_async_copy(wmod_hbm, wmod_v, sems.at[0])
    cp_x = [pltpu.make_async_copy(xT_hbm.at[:, pl.ds(128 * g, 128)], xs_v.at[g, pl.ds(0, D)], sems.at[1])
            for g in range(NG)]
    cp_xd = [pltpu.make_async_copy(xT_hbm.at[pl.ds(384, 64), pl.ds(128 * g, 128)],
                                   xs_v.at[g, pl.ds(D, 64)], sems.at[1]) for g in range(NG)]
    cp_q = [half(wq_hbm, wq_v, t, 2) for t in range(2)]
    cp_k = [half(wk_hbm, wk_v, t, 3) for t in range(2)]
    cp_v = [half(wv_hbm, wv_v, t, 4) for t in range(2)]
    cp_o = pltpu.make_async_copy(woT_hbm, wo_v, sems.at[5])
    cp_g = pltpu.make_async_copy(wg_hbm, wg_v, sems.at[6])
    cp_u = pltpu.make_async_copy(wu_hbm, wu_v, sems.at[7])
    cp_d = pltpu.make_async_copy(wdT_hbm, wd_v, sems.at[8])
    for cp in cp_q + cp_k + cp_v + [cp_o, cp_mod] + cp_x + cp_xd + [cp_g, cp_u, cp_d]:
        cp.start()

    lane = lax.broadcasted_iota(jnp.int32, (8, 128), 1)
    sub = lax.broadcasted_iota(jnp.int32, (8, 128), 0)
    low = lane < 64

    def pair_rows(buf, a, b):
        w32 = buf.bitcast(U32)
        views = [w32.at[t, pl.ds(pl.multiple_of(4 * a, 4), 8 * D - 4)] for t in range(2)]
        parts = [_unpack(v[pl.ds(b, D, stride=8), :]) for v in views]
        return (jnp.concatenate([parts[0][0], parts[1][0]], axis=1),
                jnp.concatenate([parts[0][1], parts[1][1]], axis=1))

    def fold(lhs, rhs, p, base, scale):
        low_d = lax.broadcasted_iota(jnp.int32, (D, 128), 1) < 64
        zpad = jnp.zeros((DP - D, 128), F32)

        def put(col, r):
            r = jnp.concatenate([r * scale, zpad], axis=0).astype(BF16)
            w_s[:, pl.ds(pl.multiple_of(col, 128), 128)] = pltpu.bitcast(r, U32)

        tail = jnp.concatenate([rhs[0][384:448], rhs[1][384:448]], axis=0)
        last = []
        for i in range(2):
            full = jnp.concatenate([rhs[i][0:384], tail], axis=0)
            r = lax.dot_general(lhs[i], full, NT, preferred_element_type=F32)
            for t in range(3):
                put(base + t * 2048 + (2 * p + i) * 128, r[:, 128 * t:128 * t + 128])
            last.append(r[:, 384:512])
        put(base + 3 * 2048 + p * 128, jnp.where(low_d, last[0], last[1]))

    for cp in cp_q + cp_k:
        cp.wait()

    def fold_qk(a, carry):
        for b in range(4):
            p = 4 * a + b
            q = pair_rows(wq_v, a, b)
            fold(pair_rows(wk_v, a, b), (q[0].astype(BF16), q[1].astype(BF16)), p, 0, E ** -0.5)
        return carry

    lax.fori_loop(0, 2, fold_qk, 0)
    for cp in cp_v + [cp_o]:
        cp.wait()

    def fold_vo(a, carry):
        for b in range(4):
            p = 4 * a + b
            fold(pair_rows(wv_v, a, b), (wo_v[2 * p], wo_v[2 * p + 1]), p, NW, 1.0)
        return carry

    lax.fori_loop(0, 2, fold_vo, 0)

    cp_mod.wait()
    cv = jnp.broadcast_to(c_ref[...].astype(F32), (8, D))
    mod = jnp.dot(cv * jax.nn.sigmoid(cv), wmod_v[...], preferred_element_type=F32)
    for k in range(6):
        m = _dup(mod[:, D * k:D * (k + 1)])
        vec_s[k] = 1.0 + m if k in (1, 4) else m
    vec_s[6] = _dup(jnp.broadcast_to(wr_ref[...].astype(F32), (8, D)))

    def vec(k):
        return jnp.concatenate([vec_s[k]] * (SEG // 8), axis=0)

    def load_block(q):
        g, t = q // 4, q % 4
        blk = xs_v[g, pl.ds(pl.multiple_of(t * 128, 128), 128), :].astype(F32)
        x_s[t, pl.ds(pl.multiple_of(g * 128, 128), 128), :] = blk.T

    def store_block(q):
        g, t = q // 4, q % 4
        blk = o_s[t, pl.ds(pl.multiple_of(g * 128, 128), 128), :]
        st_s[g, pl.ds(pl.multiple_of(t * 128, 128), 128), :] = blk.T.astype(BF16)

    def seg_rows(ref, s):
        r0 = pl.multiple_of(s * SEG, SEG)
        return jnp.concatenate([ref[t, pl.ds(r0, SEG), :] for t in range(4)], axis=1)

    def pre(s):
        hbuf[...] = _layernorm(seg_rows(x_s, s)) * vec(1) + vec(0)

    def post(s, valid, best, arg):
        x1 = seg_rows(x_s, s) + vec(2) * obuf[...]
        h2 = _layernorm(x1) * vec(4) + vec(3)
        out = x1 + vec(5) * h2
        r = _rowsum(h2 * vec(6))
        r0 = pl.multiple_of(s * SEG, SEG)
        for t in range(4):
            o_s[t, pl.ds(r0, SEG), :] = out[:, 128 * t:128 * t + 128]
            h2_s[t, pl.ds(r0, SEG), :] = h2[:, 128 * t:128 * t + 128]
        for g in range(SEG // 8):
            rg = jnp.broadcast_to(r[8 * g:8 * g + 8], (8, 128))
            upd = jnp.logical_and(rg > best, valid)
            best = jnp.where(upd, rg, best)
            arg = jnp.where(upd, s * SEG + 8 * g + sub, arg)
        return best, arg

    def project(hh, base, t):
        n = 2048 if t < 3 else 1024
        w = pltpu.bitcast(w_s[:, base + 2048 * t:base + 2048 * t + n], BF16)
        r = jnp.dot(hh, w, preferred_element_type=F32)
        tiles = []
        for j in range(L // 8):
            rows = r[8 * j:8 * j + 8]
            if t < 3:
                parts = [rows[:, 128 * h:128 * h + 128] for h in range(H)]
            else:
                parts = []
                for p in range(H // 2):
                    v = rows[:, 128 * p:128 * p + 128]
                    parts += [jnp.where(low, v, 0.0), jnp.where(low, 0.0, v)]
            tiles.append(jnp.concatenate(parts, axis=0).astype(BF16))
        return jnp.concatenate(tiles, axis=0)

    def softmax(sc):
        rows = []
        for g in range(L // 8):
            blk = []
            for j in range(L // 8):
                v = sc[8 * g:8 * g + 8, 128 * j:128 * j + 128]
                if g < 4 and j == g:
                    v = jnp.where((lane & 7) <= sub, v, -1e9)
                elif g < j < 4:
                    v = jnp.full((8, 128), -1e9, F32)
                blk.append(v)
            m = _group8(functools.reduce(jnp.maximum, blk), jnp.maximum, lane)
            ex = [jnp.exp(v - m) for v in blk]
            inv = 1.0 / _group8(functools.reduce(jnp.add, ex), jnp.add, lane)
            rows.append(jnp.concatenate([e * inv for e in ex], axis=1))
        return jnp.concatenate(rows, axis=0)

    for cp in cp_x + cp_xd:
        cp.wait()
    for q in range(5):
        load_block(q)
    pre(0)
    obuf[...] = jnp.zeros((SEG, DP), F32)
    for t in range(4):
        o_s[t, 0:128, :] = jnp.zeros((128, 128), F32)

    def step(s, carry):
        mem, best, arg = carry
        hh = jnp.concatenate([hbuf[...], mem], axis=0)
        kmat = jnp.concatenate([project(hh, 0, t) for t in range(4)], axis=1)
        v01 = [project(hh, NW, t) for t in range(2)]
        sc = lax.dot_general(hh, kmat, NT, preferred_element_type=F32)
        v23 = [project(hh, NW, t) for t in range(2, 4)]
        p = softmax(sc)
        best, arg = post(jnp.maximum(s - 1, 0), s > 0, best, arg)
        pre(jnp.minimum(s + 1, NSEG - 1))
        load_block(jnp.minimum(s + 5, 4 * NG - 1))
        store_block(jnp.maximum(s - 5, 0))
        o = jnp.dot(p, jnp.concatenate(v01 + v23, axis=1), preferred_element_type=F32)
        o3 = o[:, 384:512]
        o = jnp.concatenate([o[:, 0:384], o3 + pltpu.roll(o3, 64, 1)], axis=1)
        obuf[...] = o[0:SEG]
        return o[SEG:L], best, arg

    init = (_dup(mem0_ref[...].astype(F32)), jnp.full((8, 128), -jnp.inf, F32),
            jnp.zeros((8, 128), jnp.int32))
    _, best, arg = lax.fori_loop(0, NSEG, step, init)
    best, arg = post(NSEG - 1, True, best, arg)
    for q in range(4 * NG - 5, 4 * NG):
        store_block(q)

    top = jnp.max(best, axis=0, keepdims=True)
    idx = jnp.min(jnp.where(best == top, arg, S - 1))
    idx = jnp.clip(idx, 0, S - 1)
    xsel = jnp.concatenate([h2_s[t, pl.ds(idx, 1), :] for t in range(4)], axis=1)
    xsel = jnp.broadcast_to(xsel, (8, DP))[:, 0:D]
    cp_g.wait()
    cp_u.wait()
    cp_d.wait()
    gate = jnp.dot(xsel, wg_v[...], preferred_element_type=F32)
    up = jnp.dot(xsel, wu_v[...], preferred_element_type=F32)
    act = gate * jax.nn.sigmoid(gate) * up
    y = lax.dot_general(act, wd_v[...], NT, preferred_element_type=F32)
    y = _dup(y) * jax.nn.sigmoid(top[:, 0:1]) * vec_s[5]
    for t in range(4):
        o_s[t, pl.ds(idx, 1), :] = o_s[t, pl.ds(idx, 1), :] + y[0:1, 128 * t:128 * t + 128]
    for t in range(4):
        store_block((idx // 128) * 4 + t)

    cp_out = [pltpu.make_async_copy(st_s.at[g, pl.ds(0, D)], out_hbm.at[:, pl.ds(128 * g, 128)], osems.at[0])
              for g in range(NG)]
    for cp in cp_out:
        cp.start()
    for cp in cp_out:
        cp.wait()


@functools.partial(jax.jit, static_argnames=("A_seg_len",))
def pallas_adaLN_cond__memory_aug_recurrent_mem_tr__moe_arch_mod__prompt_kernel(
        A_x, A_mem0, A_Wq, A_Wk, A_Wv, A_Wo, A_seg_len, B_x, B_w_r, B_w_gate, B_w_up, B_w_down, c, w_mod):
    del B_x
    assert A_seg_len == SEG and A_x.shape == (1, S, D) and A_Wq.shape == (D, H, E)
    hbm = pl.BlockSpec(memory_space=pl.ANY)
    vmem = pl.BlockSpec(memory_space=pltpu.VMEM)
    outT = pl.pallas_call(
        _kernel,
        out_shape=jax.ShapeDtypeStruct((D, S), A_x.dtype),
        in_specs=[hbm, vmem, hbm, hbm, hbm, hbm, vmem, hbm, hbm, hbm, vmem, hbm],
        out_specs=hbm,
        scratch_shapes=[
            pltpu.VMEM((2, D * H, 128), BF16),
            pltpu.VMEM((2, D * H, 128), BF16),
            pltpu.VMEM((2, D * H, 128), BF16),
            pltpu.VMEM((H, D, E), BF16),
            pltpu.VMEM((D, 6 * D), BF16),
            pltpu.VMEM((D, FF), BF16),
            pltpu.VMEM((D, FF), BF16),
            pltpu.VMEM((D, FF), BF16),
            pltpu.VMEM((NG, DP, 128), BF16),
            pltpu.VMEM((DP // 2, 2 * NW), U32),
            pltpu.VMEM((7, 8, DP), F32),
            pltpu.VMEM((4, S, 128), F32),
            pltpu.VMEM((4, S, 128), F32),
            pltpu.VMEM((4, S, 128), F32),
            pltpu.VMEM((NG, DP, 128), BF16),
            pltpu.VMEM((SEG, DP), F32),
            pltpu.VMEM((SEG, DP), F32),
            pltpu.SemaphoreType.DMA((9,)),
            pltpu.SemaphoreType.DMA((1,)),
        ],
        compiler_params=pltpu.CompilerParams(vmem_limit_bytes=100 * 1024 * 1024),
        name="adaln_rmt_mod",
    )(
        A_x.reshape(S, D).T,
        A_mem0.reshape(M, D),
        A_Wq.reshape(D * H, E),
        A_Wk.reshape(D * H, E),
        A_Wv.reshape(D * H, E),
        A_Wo.transpose(0, 2, 1),
        B_w_r.reshape(1, D),
        B_w_gate,
        B_w_up,
        B_w_down.T,
        c,
        w_mod,
    )
    return outT.T.reshape(1, S, D)
```

```python
import functools

import jax
import jax.numpy as jnp
from jax import lax
from jax.experimental import pallas as pl
from jax.experimental.pallas import tpu as pltpu

F32 = jnp.float32
BF16 = jnp.bfloat16
U32 = jnp.uint32

S, D, H, E, M, SEG, FF = 2048, 448, 16, 256, 8, 32, 1792
DP = 512
NSEG = S // SEG
NG = S // 128
L = SEG + M
NW = H * D
NT = (((1,), (1,)), ((), ()))
EPS = 1e-5
NSEM = 45


def _dup(v):
    return jnp.concatenate([v, v[:, 384:448]], axis=1)


def _rowsum(v):
    t = v[:, 0:128] + v[:, 128:256] + v[:, 256:384] + 0.5 * v[:, 384:512]
    return jnp.sum(t, axis=1, keepdims=True)


def _layernorm(v):
    mu = _rowsum(v) * (1.0 / D)
    d = v - mu
    var = _rowsum(d * d) * (1.0 / D)
    return d * lax.rsqrt(var + EPS)


def _group8(v, op, lane):
    for d in (1, 2, 4):
        up = pltpu.roll(v, d, 1)
        dn = pltpu.roll(v, 128 - d, 1)
        v = op(v, jnp.where((lane & d) != 0, up, dn))
    return v


def _unpack(u):
    lo = pltpu.bitcast(u << 16, F32)
    hi = pltpu.bitcast(u & jnp.uint32(0xFFFF0000), F32)
    return lo, hi


def _kernel(xT_hbm, mem0_hbm, wq_hbm, wk_hbm, wv_hbm, woT_hbm, wr_hbm, wg_hbm, wu_hbm, wdT_hbm,
            c_hbm, wmod_hbm, out_hbm, mem0_ref, wr_ref, c_ref,
            wq_v, wk_v, kh_s, wv_v, wo_v, wmod_v, wg_v, wu_v, wd_v, xs_v, wk1_s, wq2_s, wv1_s, wb2_s, vec_s,
            x_s, o_s, h2_s, st_s, sems, osem):
    sem_ids = iter(range(NSEM))

    def copy(src, dst, k=None):
        return pltpu.make_async_copy(src, dst, sems.at[next(sem_ids) if k is None else k])

    def halves(src, dst, r0, n):
        return [copy(src.at[pl.ds(r0, n), pl.ds(128 * t, 128)], dst.at[t, pl.ds(r0, n)]) for t in range(2)]

    def x_group(g, k=None):
        cols = pl.ds(128 * g, 128)
        return [copy(xT_hbm.at[:, cols], xs_v.at[g, pl.ds(0, D)], k),
                copy(xT_hbm.at[pl.ds(384, 64), cols], xs_v.at[g, pl.ds(D, 64)], k)]

    cp_k = [halves(wk_hbm, wk_v, 64 * H * i, 64 * H) for i in range(D // 64)]
    cp_q = [halves(wq_hbm, wq_v, 128 * H * t, (128 if t < 3 else 64) * H) for t in range(4)]
    cp_v = halves(wv_hbm, wv_v, 0, D * H)
    cp_o = [copy(woT_hbm.at[pl.ds(2 * p, 2)], wo_v.at[pl.ds(2 * p, 2)]) for p in range(H // 2)]
    cp_x0 = x_group(0) + x_group(1)
    cp_mod = [copy(c_hbm, c_ref), copy(wr_hbm, wr_ref), copy(mem0_hbm, mem0_ref), copy(wmod_hbm, wmod_v)]
    k_x = next(sem_ids)
    cp_x = [cp for g in range(2, NG) for cp in x_group(g, k_x)]
    cp_ffn = [copy(wg_hbm, wg_v), copy(wu_hbm, wu_v), copy(wdT_hbm, wd_v)]
    for cp in sum(cp_k, []) + sum(cp_q, []) + cp_v + cp_o + cp_x0 + cp_mod + cp_x + cp_ffn:
        cp.start()

    lane = lax.broadcasted_iota(jnp.int32, (8, 128), 1)
    sub = lax.broadcasted_iota(jnp.int32, (8, 128), 0)
    low = lane < 64
    low64 = lax.broadcasted_iota(jnp.int32, (64, 128), 1) < 64

    def pair_rows(buf, p, d0, n):
        w32 = buf.bitcast(U32)
        views = [w32.at[t, pl.ds(pl.multiple_of(8 * d0, 8), 8 * n)] for t in range(2)]
        parts = [_unpack(v[pl.ds(p, n, stride=8), :]) for v in views]
        return [jnp.concatenate([parts[0][i], parts[1][i]], axis=1) for i in range(2)]

    def packed(r):
        return pltpu.bitcast(r.astype(BF16), U32)

    def slab(col):
        return pl.ds(pl.multiple_of(col, 128), 128)

    def fold_main(lhs, rhs, t, p, dst, scale):
        rest = []
        for i in range(2):
            r = lax.dot_general(lhs[i], rhs[i].astype(BF16), NT, preferred_element_type=F32) * scale
            c0 = t * 2048 + (2 * p + i) * 128
            dst[:, c0:c0 + 128] = packed(r[0:384])
            rest.append(r[384:448])
        return jnp.concatenate(rest, axis=0)

    def fold_tail(lhs, rhs, p, dst, scale):
        both = jnp.concatenate([lhs[0][384:448], lhs[1][384:448]], axis=0)
        r = jnp.concatenate(
            [lax.dot_general(rhs[i], jnp.concatenate([lhs[i][0:384], both], axis=0).astype(BF16), NT,
                             preferred_element_type=F32) for i in range(2)], axis=0) * scale
        dst[:, 3 * 2048 + p * 128:3 * 2048 + p * 128 + 128] = packed(r[:, 0:384].T)
        return r[:, 384:512]

    def split_k(i, carry):
        for ii in range(D // 64):
            @pl.when(i == ii)
            def _():
                for cp in cp_k[ii]:
                    cp.wait()
        for p in range(H // 2):
            rows = pair_rows(wk_v, p, 64 * i, 64)
            for h in range(2):
                kh_s[2 * p + h, pl.ds(pl.multiple_of(32 * i, 32), 32), :] = packed(rows[h])
        return carry

    lax.fori_loop(0, D // 64, split_k, 0)

    def heads_k(p):
        return [pltpu.bitcast(kh_s[2 * p + h], BF16) for h in range(2)]

    def fold_qk(t, p):
        k = heads_k(p)
        rest = fold_main(k, pair_rows(wq_v, p, 128 * t, 128), t, p, wk1_s, E ** -0.5)
        wq2_s[64 * t:64 * t + 64, 128 * p:128 * p + 128] = packed(rest.T)
        if t == 2:
            r = fold_tail(k, pair_rows(wq_v, p, 384, 64), p, wk1_s, E ** -0.5)
            r = jnp.concatenate([jnp.where(low64, r[0:64], r[64:128]), jnp.zeros((64, 128), F32)], axis=0)
            wq2_s[192:256, 128 * p:128 * p + 128] = packed(r)

    def fold_vo(p):
        v = pair_rows(wv_v, p, 0, D)
        for t in range(3):
            rest = fold_main(v, [wo_v[2 * p + i, 128 * t:128 * t + 128, :] for i in range(2)], t, p, wv1_s, 1.0)
            wb2_s[64 * p:64 * p + 64, 128 * t:128 * t + 128] = packed(rest)
        r = fold_tail(v, [wo_v[2 * p + i, 384:448, :].astype(F32) for i in range(2)], p, wv1_s, 1.0).T
        o = pltpu.roll(r, 64, 1)
        wb2_s[64 * p:64 * p + 64, 384:512] = packed(jnp.concatenate(
            [jnp.where(low64, r[0:64], o[0:64]), jnp.where(low64, o[64:128], r[64:128])], axis=0))

    for t, needs in enumerate((cp_q[0], cp_q[1], cp_q[2] + cp_q[3])):
        for cp in needs:
            cp.wait()
        for p in range(H // 2):
            fold_qk(t, p)
    for cp in cp_v:
        cp.wait()
    for pairs in ((0,), (1, 2), (3, 4, 5, 6)):
        for p in pairs:
            cp_o[p].wait()
        for p in pairs:
            fold_vo(p)
    cp_o[7].wait()

    for cp in cp_x0 + cp_mod:
        cp.wait()
    cv = jnp.broadcast_to(c_ref[...].astype(F32), (8, D))
    mod = jnp.dot(cv * jax.nn.sigmoid(cv), wmod_v[...], preferred_element_type=F32)
    for k in range(6):
        m = _dup(mod[:, D * k:D * (k + 1)])
        vec_s[k] = 1.0 + m if k in (1, 4) else m
    vec_s[6] = _dup(jnp.broadcast_to(wr_ref[...].astype(F32).reshape(1, D), (8, D)))

    def vec(k):
        return jnp.concatenate([vec_s[k]] * (SEG // 8), axis=0)

    def rows_of(g):
        return pl.ds(pl.multiple_of(g * 128, 128), 128)

    def load_group(g, ts=range(4)):
        for t in ts:
            x_s[t, rows_of(g), :] = xs_v[g, 128 * t:128 * t + 128, :].astype(F32).T

    def store_group(g, ts=range(4)):
        for t in ts:
            st_s[g, 128 * t:128 * t + 128, :] = o_s[t, rows_of(g), :].T.astype(BF16)

    def seg_rows(ref, s):
        r0 = pl.multiple_of(s * SEG, SEG)
        return jnp.concatenate([ref[t, pl.ds(r0, SEG), :] for t in range(4)], axis=1)

    def pre(s):
        h = _layernorm(seg_rows(x_s, s)) * vec(1) + vec(0)
        for t in range(4):
            (o_s, h2_s)[t // 2][t % 2, S:S + SEG, :] = h[:, 128 * t:128 * t + 128]

    def parked():
        return jnp.concatenate([(o_s, h2_s)[t // 2][t % 2, S:S + SEG, :] for t in range(4)], axis=1)

    def post(s, attn, valid, best, arg):
        x1 = seg_rows(x_s, s) + vec(2) * attn
        h2 = _layernorm(x1) * vec(4) + vec(3)
        out = x1 + vec(5) * h2
        r = _rowsum(h2 * vec(6))
        r0 = pl.multiple_of(s * SEG, SEG)
        for t in range(4):
            o_s[t, pl.ds(r0, SEG), :] = out[:, 128 * t:128 * t + 128]
            h2_s[t, pl.ds(r0, SEG), :] = h2[:, 128 * t:128 * t + 128]
        for g in range(SEG // 8):
            rg = jnp.broadcast_to(r[8 * g:8 * g + 8], (8, 128))
            upd = jnp.logical_and(rg > best, valid)
            best = jnp.where(upd, rg, best)
            arg = jnp.where(upd, s * SEG + 8 * g + sub, arg)
        return best, arg

    def project(h1, w_ref, t, h0, hn, dup):
        w = 128 if t < 3 else 64
        c0 = 2048 * t + w * h0
        r = jnp.dot(h1, pltpu.bitcast(w_ref[:, c0:c0 + w * (hn - h0)], BF16), preferred_element_type=F32)
        tiles = []
        for j in range(L // 8):
            rows = r[8 * j:8 * j + 8]
            if t < 3:
                parts = [rows[:, 128 * h:128 * h + 128] for h in range(hn - h0)]
            else:
                parts = []
                for p in range((hn - h0) // 2):
                    v = rows[:, 128 * p:128 * p + 128]
                    o = pltpu.roll(v, 64, 1) if dup else 0.0
                    parts += [jnp.where(low, v, o), jnp.where(low, o, v)]
            tiles.append(jnp.concatenate(parts, axis=0))
        return tiles

    def barrel(src, want):
        def stage(k, c):
            if k < 0:
                return src[c]
            key = (k, c)
            if key not in memo:
                hi, lo = stage(k - 1, (c + (1 << k)) % 8), stage(k - 1, c)
                memo[key] = lo if hi is None else hi if lo is None else jnp.where((lane & (16 << k)) != 0, hi, lo)
            return memo[key]
        memo = {}
        return [stage(2, c) for c in want]

    def softmax(sc, tt):
        p_rows, z_rows = [], []
        for g in (4, 0, 1, 2, 3):
            extra = barrel([t[8 * g:8 * g + 8] for t in tt], [(-j) % 8 for j in range(L // 8)])
            blk = []
            for j in range(L // 8):
                if g < j < 4:
                    blk.append(jnp.full((8, 128), -1e9, F32))
                    continue
                r0 = 8 * (g - j) if j < SEG // 8 else 8 * g
                v = sc[j][r0:r0 + 8] + (pltpu.roll(extra[j], 128 - 16 * j, 1) if j else extra[j])
                if g < 4 and j == g:
                    v = jnp.where((lane & 7) <= sub, v, -1e9)
                blk.append(v)
            m = _group8(functools.reduce(jnp.maximum, blk), jnp.maximum, lane)
            ex = [jnp.exp(v - m) for v in blk]
            inv = 1.0 / _group8(functools.reduce(jnp.add, ex), jnp.add, lane)
            pr = [e * inv for e in ex]
            p_rows.append(jnp.concatenate(pr, axis=1))
            rolled = [pltpu.roll(v, 16 * j, 1) if j else v for j, v in enumerate(pr)]
            z_rows.append(jnp.concatenate(barrel(rolled + [None] * 3, [(-i) % 8 for i in range(8)]), axis=1))
        return jnp.concatenate(p_rows, axis=0), jnp.concatenate(z_rows, axis=0)

    load_group(0)
    load_group(1)
    pre(0)
    for t in range(4):
        o_s[t, 0:128, :] = jnp.zeros((128, 128), F32)
    fold_vo(7)
    for cp in cp_x:
        cp.wait()

    def out_copy(g):
        return pltpu.make_async_copy(st_s.at[g, pl.ds(0, D)], out_hbm.at[:, slab(g * 128)], osem.at[0])

    def step(s, carry):
        mem, attn, best, arg = carry
        hh = jnp.concatenate([parked(), mem], axis=0)
        h1 = hh[:, 0:384]
        best, arg = post(jnp.maximum(s - 1, 0), attn, s > 0, best, arg)
        pre(jnp.minimum(s + 1, NSEG - 1))

        tails = []
        for j in range(L // 8):
            v = hh[8 * j:8 * j + 8, 384:512]
            tails.append(jnp.concatenate([jnp.where(low, v, 0.0), jnp.where(low, 0.0, v)], axis=0))
        tails += [jnp.zeros((16, 128), F32)] * 3
        tail_rhs = [jnp.concatenate([tails[(b - i) % 8] for b in range(8)], axis=0).astype(BF16)
                    for i in range(8)]

        q2 = jnp.dot(hh, pltpu.bitcast(wq2_s[...], BF16), preferred_element_type=F32)
        vt = [[] for _ in range(4)]
        todo = [(t, h) for t in (3, 0, 1, 2) for h in range(0, H, 4 if t < 3 else 8)]

        def next_v():
            t, h = todo.pop(0)
            vt[t].append(project(h1, wv1_s, t, h, h + (4 if t < 3 else 8), True))

        sc = [None] * (L // 8)
        tt = []

        def tail_scores(pairs):
            for i in pairs:
                tt.append(lax.dot_general(q2[:, 128 * i:128 * i + 128], tail_rhs[i], NT,
                                          preferred_element_type=F32))

        def scores(kt, t, groups):
            for j in groups:
                r0 = 8 * j if j < SEG // 8 else 0
                d = lax.dot_general(hh[r0:, 128 * t:128 * t + 128], kt[j].astype(BF16), NT,
                                    preferred_element_type=F32)
                sc[j] = d if sc[j] is None else sc[j] + d

        def keys(t, between):
            a = project(h1, wk1_s, t, 0, H // 2, False)
            between()
            b = project(h1, wk1_s, t, H // 2, H, False)
            return [jnp.concatenate([x, y], axis=0) for x, y in zip(a, b)]

        k3 = project(h1, wk1_s, 3, 0, H, False)
        k0 = keys(0, lambda: tail_scores(range(4)))
        scores(k3, 3, (4, 0, 1, 2))
        k1 = keys(1, lambda: tail_scores(range(4, 8)))
        scores(k0, 0, (4, 0, 1, 2))
        k2 = keys(2, lambda: (scores(k3, 3, (3,)), scores(k0, 0, (3,)), scores(k1, 1, (3, 4))))
        scores(k1, 1, (0, 1, 2))
        next_v()
        next_v()
        scores(k2, 2, (4,))
        next_v()
        scores(k2, 2, (0, 1, 2, 3))
        p, z = softmax(sc, tt)
        while todo:
            next_v()
        u = jnp.concatenate([jnp.dot(z[:, 128 * i:128 * i + 128], tail_rhs[i], preferred_element_type=F32)
                             for i in range(8)], axis=1)
        vmat = jnp.concatenate(
            [jnp.concatenate([piece[j] for j in range(L // 8) for piece in vt[t]], axis=0) for t in range(4)],
            axis=1)
        o = jnp.dot(p, vmat.astype(BF16), preferred_element_type=F32)
        o = jnp.dot(u, pltpu.bitcast(wb2_s[...], BF16), preferred_element_type=F32) + o
        return o[0:M], o[M:L], best, arg

    def group(g, carry):
        @pl.when(g >= 3)
        def _():
            out_copy(g - 3).start()

        for i in range(4):
            carry = step(4 * g + i, carry)
            store_group(jnp.maximum(g - 2, 0), (i,))
            load_group(jnp.minimum(g + 2, NG - 1), (i,))
        return carry

    init = (_dup(mem0_ref[...].astype(F32)), jnp.zeros((SEG, DP), F32),
            jnp.full((8, 128), -jnp.inf, F32), jnp.zeros((8, 128), jnp.int32))
    _, attn, best, arg = lax.fori_loop(0, NG, group, init)
    for cp in cp_ffn:
        cp.wait()
    best, arg = post(NSEG - 1, attn, True, best, arg)

    top = jnp.max(best, axis=0, keepdims=True)
    idx = jnp.min(jnp.where(best == top, arg, S - 1))
    idx = jnp.clip(idx, 0, S - 1)
    xsel = jnp.concatenate([h2_s[t, pl.ds(idx, 1), :] for t in range(4)], axis=1)
    xsel = jnp.broadcast_to(xsel, (8, DP))[:, 0:D]
    store_group(NG - 2)
    store_group(NG - 1)
    gate = jnp.dot(xsel, wg_v[...], preferred_element_type=F32)
    up = jnp.dot(xsel, wu_v[...], preferred_element_type=F32)
    for g in range(NG - 3, NG):
        out_copy(g).start()
    act = gate * jax.nn.sigmoid(gate) * up
    y = lax.dot_general(act, wd_v[...], NT, preferred_element_type=F32)
    y = _dup(y) * jax.nn.sigmoid(top[:, 0:1]) * vec_s[5]
    for t in range(4):
        o_s[t, pl.ds(idx, 1), :] = o_s[t, pl.ds(idx, 1), :] + y[0:1, 128 * t:128 * t + 128]
    for g in range(NG):
        out_copy(g).wait()
    store_group(idx // 128)
    patch = out_copy(idx // 128)
    patch.start()
    patch.wait()


@functools.partial(jax.jit, static_argnames=("A_seg_len",))
def pallas_adaLN_cond__memory_aug_recurrent_mem_tr__moe_arch_mod__prompt_kernel(
        A_x, A_mem0, A_Wq, A_Wk, A_Wv, A_Wo, A_seg_len, B_x, B_w_r, B_w_gate, B_w_up, B_w_down, c, w_mod):
    del B_x
    assert A_seg_len == SEG and A_x.shape == (1, S, D) and A_Wq.shape == (D, H, E)
    hbm = pl.BlockSpec(memory_space=pl.ANY)
    outT = pl.pallas_call(
        _kernel,
        out_shape=jax.ShapeDtypeStruct((D, S), A_x.dtype),
        in_specs=[hbm] * 12,
        out_specs=hbm,
        scratch_shapes=[
            pltpu.VMEM((M, D), BF16),
            pltpu.VMEM((D,), BF16),
            pltpu.VMEM((1, D), BF16),
            pltpu.VMEM((2, D * H, 128), BF16),
            pltpu.VMEM((2, D * H, 128), BF16),
            pltpu.VMEM((H, D // 2, E), U32),
            pltpu.VMEM((2, D * H, 128), BF16),
            pltpu.VMEM((H, D, E), BF16),
            pltpu.VMEM((D, 6 * D), BF16),
            pltpu.VMEM((D, FF), BF16),
            pltpu.VMEM((D, FF), BF16),
            pltpu.VMEM((D, FF), BF16),
            pltpu.VMEM((NG, DP, 128), BF16),
            pltpu.VMEM((192, NW), U32),
            pltpu.VMEM((DP // 2, 64 * H), U32),
            pltpu.VMEM((192, NW), U32),
            pltpu.VMEM((32 * H, DP), U32),
            pltpu.VMEM((7, 8, DP), F32),
            pltpu.VMEM((4, S, 128), F32),
            pltpu.VMEM((4, S + SEG, 128), F32),
            pltpu.VMEM((4, S + SEG, 128), F32),
            pltpu.VMEM((NG, DP, 128), BF16),
            pltpu.SemaphoreType.DMA((NSEM,)),
            pltpu.SemaphoreType.DMA((1,)),
        ],
        compiler_params=pltpu.CompilerParams(vmem_limit_bytes=100 * 1024 * 1024),
        name="adaln_rmt_mod",
    )(
        A_x.reshape(S, D).T,
        A_mem0.reshape(M, D),
        A_Wq.reshape(D * H, E),
        A_Wk.reshape(D * H, E),
        A_Wv.reshape(D * H, E),
        A_Wo.transpose(0, 2, 1),
        B_w_r,
        B_w_gate,
        B_w_up,
        B_w_down.T,
        c,
        w_mod,
    )
    return outT.T.reshape(1, S, D)
```

```python
import functools

import jax
import jax.numpy as jnp
from jax import lax
from jax.experimental import pallas as pl
from jax.experimental.pallas import tpu as pltpu

F32 = jnp.float32
BF16 = jnp.bfloat16
U32 = jnp.uint32

S, D, H, E, M, SEG, FF = 2048, 448, 16, 256, 8, 32, 1792
DP = 512
NSEG = S // SEG
NG = S // 128
L = SEG + M
NW = H * D
NT = (((1,), (1,)), ((), ()))
EPS = 1e-5
NSEM = 21


def _dup(v):
    return jnp.concatenate([v, v[:, 384:448]], axis=1)


def _rowsum(v):
    t = v[:, 0:128] + v[:, 128:256] + v[:, 256:384] + 0.5 * v[:, 384:512]
    return jnp.sum(t, axis=1, keepdims=True)


def _layernorm(v):
    mu = _rowsum(v) * (1.0 / D)
    d = v - mu
    var = _rowsum(d * d) * (1.0 / D)
    return d * lax.rsqrt(var + EPS)


def _group8(v, op, lane):
    for d in (1, 2, 4):
        up = pltpu.roll(v, d, 1)
        dn = pltpu.roll(v, 128 - d, 1)
        v = op(v, jnp.where((lane & d) != 0, up, dn))
    return v


def _unpack(u):
    lo = pltpu.bitcast(u << 16, F32)
    hi = pltpu.bitcast(u & jnp.uint32(0xFFFF0000), F32)
    return lo, hi


def _kernel(xT_hbm, mem0_hbm, wq_hbm, wk_hbm, wv_hbm, woT_hbm, wr_hbm, wg_hbm, wu_hbm, wdT_hbm,
            c_hbm, wmod_hbm, out_hbm, mem0_ref, wr_ref, c_ref,
            wq_v, wk_v, wv_v, wo_v, acc_s, acct_s, wmod_v, wg_v, wu_v, wd_v, xs_v, wk1_s, wq2_s, wv1_s, wb2_s, vec_s,
            x_s, o_s, h2_s, st_s, sems, osem):
    sem_ids = iter(range(NSEM))

    def copy(src, dst):
        return pltpu.make_async_copy(src, dst, sems.at[next(sem_ids)])

    def slab(col):
        return pl.ds(pl.multiple_of(col, 128), 128)

    def x_group(g, k):
        cols = pl.ds(128 * g, 128)
        return [pltpu.make_async_copy(xT_hbm.at[:, cols], xs_v.at[g, pl.ds(0, D)], sems.at[k]),
                pltpu.make_async_copy(xT_hbm.at[pl.ds(384, 64), cols], xs_v.at[g, pl.ds(D, 64)], sems.at[k])]

    def rows_copy(src, dst, e, d0, n):
        return copy(src.at[pl.ds(H * d0, H * n), pl.ds(128 * e, 128)], dst.at[e, pl.ds(H * d0, H * n)])

    cp_qk = [[[rows_copy(wk_hbm, wk_v, e, 0, D), rows_copy(wq_hbm, wq_v, e, 0, 256)],
              [rows_copy(wq_hbm, wq_v, e, 256, D - 256)]] for e in range(2)]

    def wo_copy(e, a):
        hs = pl.ds(8 * a, 8)
        return copy(woT_hbm.at[hs, :, pl.ds(128 * e, 128)], wo_v.at[e, hs])

    cp_vo = [[[rows_copy(wv_hbm, wv_v, e, 0, D), wo_copy(e, 0)], [wo_copy(e, 1)]] for e in range(2)]
    k_x0, k_x = next(sem_ids), next(sem_ids)
    cp_x0 = [cp for g in range(3) for cp in x_group(g, k_x0)]
    cp_mod = [copy(c_hbm, c_ref), copy(wr_hbm, wr_ref), copy(mem0_hbm, mem0_ref), copy(wmod_hbm, wmod_v)]
    cp_x = [cp for g in range(3, NG) for cp in x_group(g, k_x)]
    cp_ffn = [copy(wg_hbm, wg_v), copy(wu_hbm, wu_v), copy(wdT_hbm, wd_v)]
    for cp in sum(sum(cp_qk + cp_vo, []), []) + cp_x0 + cp_mod + cp_x + cp_ffn:
        cp.start()

    lane = lax.broadcasted_iota(jnp.int32, (8, 128), 1)
    sub = lax.broadcasted_iota(jnp.int32, (8, 128), 0)
    low = lane < 64
    low64 = lax.broadcasted_iota(jnp.int32, (64, 128), 1) < 64

    def pair_rows(buf, e, p, d0, n):
        view = buf.bitcast(U32).at[e, pl.ds(8 * d0, 8 * n)]
        return _unpack(view[pl.ds(p, n, stride=8), :])

    def packed(r):
        return pltpu.bitcast(r.astype(BF16), U32)

    def fold_main(lhs, rhs, e, t, p, dst, scale):
        rest = []
        for i in range(2):
            r = lax.dot_general(lhs[i], rhs[i].astype(BF16), NT, preferred_element_type=F32)
            if e == 0:
                acc_s[2 * p + i, t] = r
                continue
            r = (r + acc_s[2 * p + i, t]) * scale
            c0 = t * 2048 + (2 * p + i) * 128
            dst[:, c0:c0 + 128] = packed(r[0:384])
            rest.append(r[384:448])
        return jnp.concatenate(rest, axis=0) if e else None

    def fold_tail(lhs, rhs, e, p, dst, scale):
        both = jnp.concatenate([lhs[0][384:448], lhs[1][384:448]], axis=0)
        r = jnp.concatenate(
            [lax.dot_general(rhs[i], jnp.concatenate([lhs[i][0:384], both], axis=0).astype(BF16), NT,
                             preferred_element_type=F32) for i in range(2)], axis=0)
        if e == 0:
            acct_s[p] = r
            return None
        r = (r + acct_s[p]) * scale
        dst[:, 3 * 2048 + p * 128:3 * 2048 + p * 128 + 128] = packed(r[:, 0:384].T)
        return r[:, 384:512]

    def fold_qk(e, part, p):
        k = pair_rows(wk_v, e, p, 0, D)
        for t in ((0, 1), (2,))[part]:
            rest = fold_main(k, pair_rows(wq_v, e, p, 128 * t, 128), e, t, p, wk1_s, E ** -0.5)
            if e:
                wq2_s[64 * t:64 * t + 64, 128 * p:128 * p + 128] = packed(rest.T)
        if part:
            r = fold_tail(k, pair_rows(wq_v, e, p, 384, 64), e, p, wk1_s, E ** -0.5)
            if e:
                r = jnp.concatenate([jnp.where(low64, r[0:64], r[64:128]), jnp.zeros((64, 128), F32)], axis=0)
                wq2_s[192:256, 128 * p:128 * p + 128] = packed(r)

    def fold_vo(e, p):
        v = pair_rows(wv_v, e, p, 0, D)
        for t in range(3):
            rest = fold_main(v, [wo_v[e, 2 * p + i, 128 * t:128 * t + 128, :] for i in range(2)],
                             e, t, p, wv1_s, 1.0)
            if e:
                wb2_s[64 * p:64 * p + 64, 128 * t:128 * t + 128] = packed(rest)
        r = fold_tail(v, [wo_v[e, 2 * p + i, 384:448, :].astype(F32) for i in range(2)], e, p, wv1_s, 1.0)
        if e:
            r = r.T
            o = pltpu.roll(r, 64, 1)
            wb2_s[64 * p:64 * p + 64, 384:512] = packed(jnp.concatenate(
                [jnp.where(low64, r[0:64], o[0:64]), jnp.where(low64, o[64:128], r[64:128])], axis=0))

    for e in range(2):
        for part in range(2):
            for cp in cp_qk[e][part]:
                cp.wait()
            for p in range(H // 2):
                fold_qk(e, part, p)
    for e in range(2):
        for a in range(2):
            for cp in cp_vo[e][a]:
                cp.wait()
            for p in range(4 * a, 4 * a + 4):
                fold_vo(e, p)

    for cp in cp_x0 + cp_mod:
        cp.wait()
    cv = jnp.broadcast_to(c_ref[...].astype(F32), (8, D))
    mod = jnp.dot(cv * jax.nn.sigmoid(cv), wmod_v[...], preferred_element_type=F32)
    for k in range(6):
        m = _dup(mod[:, D * k:D * (k + 1)])
        vec_s[k] = 1.0 + m if k in (1, 4) else m
    vec_s[6] = _dup(jnp.broadcast_to(wr_ref[...].astype(F32).reshape(1, D), (8, D)))

    def vec(k):
        return jnp.concatenate([vec_s[k]] * (SEG // 8), axis=0)

    def rows_of(g):
        return pl.ds(pl.multiple_of(g * 128, 128), 128)

    def load_group(g, ts=range(4)):
        for t in ts:
            x_s[t, rows_of(g), :] = xs_v[g, 128 * t:128 * t + 128, :].astype(F32).T

    def store_group(g, ts=range(4)):
        for t in ts:
            st_s[g, 128 * t:128 * t + 128, :] = o_s[t, rows_of(g), :].T.astype(BF16)

    def seg_rows(ref, s):
        r0 = pl.multiple_of(s * SEG, SEG)
        return jnp.concatenate([ref[t, pl.ds(r0, SEG), :] for t in range(4)], axis=1)

    def pre(s):
        h = _layernorm(seg_rows(x_s, s)) * vec(1) + vec(0)
        for t in range(4):
            (o_s, h2_s)[t // 2][t % 2, S:S + SEG, :] = h[:, 128 * t:128 * t + 128]

    def parked():
        return jnp.concatenate([(o_s, h2_s)[t // 2][t % 2, S:S + SEG, :] for t in range(4)], axis=1)

    def post(s, attn, valid, best, arg):
        x1 = seg_rows(x_s, s) + vec(2) * attn
        h2 = _layernorm(x1) * vec(4) + vec(3)
        out = x1 + vec(5) * h2
        r = _rowsum(h2 * vec(6))
        r0 = pl.multiple_of(s * SEG, SEG)
        for t in range(4):
            o_s[t, pl.ds(r0, SEG), :] = out[:, 128 * t:128 * t + 128]
            h2_s[t, pl.ds(r0, SEG), :] = h2[:, 128 * t:128 * t + 128]
        for g in range(SEG // 8):
            rg = jnp.broadcast_to(r[8 * g:8 * g + 8], (8, 128))
            upd = jnp.logical_and(rg > best, valid)
            best = jnp.where(upd, rg, best)
            arg = jnp.where(upd, s * SEG + 8 * g + sub, arg)
        return best, arg

    def project(h1, w_ref, t, h0, hn, dup):
        w = 128 if t < 3 else 64
        c0 = 2048 * t + w * h0
        r = jnp.dot(h1, pltpu.bitcast(w_ref[:, c0:c0 + w * (hn - h0)], BF16), preferred_element_type=F32)
        tiles = []
        for j in range(L // 8):
            rows = r[8 * j:8 * j + 8]
            if t < 3:
                parts = [rows[:, 128 * h:128 * h + 128] for h in range(hn - h0)]
            else:
                parts = []
                for p in range((hn - h0) // 2):
                    v = rows[:, 128 * p:128 * p + 128]
                    o = pltpu.roll(v, 64, 1) if dup else 0.0
                    parts += [jnp.where(low, v, o), jnp.where(low, o, v)]
            tiles.append(jnp.concatenate(parts, axis=0))
        return tiles

    def barrel(src, want):
        def stage(k, c):
            if k < 0:
                return src[c]
            key = (k, c)
            if key not in memo:
                hi, lo = stage(k - 1, (c + (1 << k)) % 8), stage(k - 1, c)
                memo[key] = lo if hi is None else hi if lo is None else jnp.where((lane & (16 << k)) != 0, hi, lo)
            return memo[key]
        memo = {}
        return [stage(2, c) for c in want]

    def softmax(sc, tt):
        p_rows, z_rows = [], []
        for g in (4, 0, 1, 2, 3):
            extra = barrel([t[8 * g:8 * g + 8] for t in tt], [(-j) % 8 for j in range(L // 8)])
            blk = []
            for j in range(L // 8):
                if g < j < 4:
                    blk.append(jnp.full((8, 128), -1e9, F32))
                    continue
                r0 = 8 * (g - j) if j < SEG // 8 else 8 * g
                v = sc[j][r0:r0 + 8] + (pltpu.roll(extra[j], 128 - 16 * j, 1) if j else extra[j])
                if g < 4 and j == g:
                    v = jnp.where((lane & 7) <= sub, v, -1e9)
                blk.append(v)
            m = _group8(functools.reduce(jnp.maximum, blk), jnp.maximum, lane)
            ex = [jnp.exp(v - m) for v in blk]
            inv = 1.0 / _group8(functools.reduce(jnp.add, ex), jnp.add, lane)
            pr = [e * inv for e in ex]
            p_rows.append(jnp.concatenate(pr, axis=1))
            rolled = [pltpu.roll(v, 16 * j, 1) if j else v for j, v in enumerate(pr)]
            z_rows.append(jnp.concatenate(barrel(rolled + [None] * 3, [(-i) % 8 for i in range(8)]), axis=1))
        return jnp.concatenate(p_rows, axis=0), jnp.concatenate(z_rows, axis=0)

    load_group(0)
    load_group(1)
    pre(0)
    for t in range(4):
        o_s[t, 0:128, :] = jnp.zeros((128, 128), F32)

    def out_copy(g):
        return pltpu.make_async_copy(st_s.at[g, pl.ds(0, D)], out_hbm.at[:, slab(g * 128)], osem.at[0])

    def step(s, carry):
        mem, attn, best, arg = carry
        hh = jnp.concatenate([parked(), mem], axis=0)
        h1 = hh[:, 0:384]
        best, arg = post(jnp.maximum(s - 1, 0), attn, s > 0, best, arg)
        pre(jnp.minimum(s + 1, NSEG - 1))

        tails = []
        for j in range(L // 8):
            v = hh[8 * j:8 * j + 8, 384:512]
            tails.append(jnp.concatenate([jnp.where(low, v, 0.0), jnp.where(low, 0.0, v)], axis=0))
        tails += [jnp.zeros((16, 128), F32)] * 3
        tail_rhs = [jnp.concatenate([tails[(b - i) % 8] for b in range(8)], axis=0).astype(BF16)
                    for i in range(8)]

        q2 = jnp.dot(hh, pltpu.bitcast(wq2_s[...], BF16), preferred_element_type=F32)
        vt = [[] for _ in range(4)]
        todo = [(t, h) for t in (3, 0, 1, 2) for h in range(0, H, 4 if t < 3 else 8)]

        def next_v():
            t, h = todo.pop(0)
            vt[t].append(project(h1, wv1_s, t, h, h + (4 if t < 3 else 8), True))

        sc = [None] * (L // 8)
        tt = []

        def tail_scores(pairs):
            for i in pairs:
                tt.append(lax.dot_general(q2[:, 128 * i:128 * i + 128], tail_rhs[i], NT,
                                          preferred_element_type=F32))

        def scores(kt, t, groups):
            for j in groups:
                r0 = 8 * j if j < SEG // 8 else 0
                d = lax.dot_general(hh[r0:, 128 * t:128 * t + 128], kt[j].astype(BF16), NT,
                                    preferred_element_type=F32)
                sc[j] = d if sc[j] is None else sc[j] + d

        def keys(t, between):
            a = project(h1, wk1_s, t, 0, H // 2, False)
            between()
            b = project(h1, wk1_s, t, H // 2, H, False)
            return [jnp.concatenate([x, y], axis=0) for x, y in zip(a, b)]

        k3 = project(h1, wk1_s, 3, 0, H, False)
        k0 = keys(0, lambda: tail_scores(range(4)))
        scores(k3, 3, (4, 0, 1, 2))
        k1 = keys(1, lambda: tail_scores(range(4, 8)))
        scores(k0, 0, (4, 0, 1, 2))
        k2 = keys(2, lambda: (scores(k3, 3, (3,)), scores(k0, 0, (3,)), scores(k1, 1, (3, 4))))
        scores(k1, 1, (0, 1, 2))
        next_v()
        next_v()
        scores(k2, 2, (4,))
        next_v()
        scores(k2, 2, (0, 1, 2, 3))
        p, z = softmax(sc, tt)
        while todo:
            next_v()
        u = jnp.concatenate([jnp.dot(z[:, 128 * i:128 * i + 128], tail_rhs[i], preferred_element_type=F32)
                             for i in range(8)], axis=1)
        vmat = jnp.concatenate(
            [jnp.concatenate([piece[j] for j in range(L // 8) for piece in vt[t]], axis=0) for t in range(4)],
            axis=1)
        o = jnp.dot(p, vmat.astype(BF16), preferred_element_type=F32)
        o = jnp.dot(u, pltpu.bitcast(wb2_s[...], BF16), preferred_element_type=F32) + o
        return o[0:M], o[M:L], best, arg

    def group(g, carry):
        @pl.when(g >= 3)
        def _():
            out_copy(g - 3).start()

        @pl.when(g == 1)
        def _():
            for cp in cp_x:
                cp.wait()

        for i in range(4):
            carry = step(4 * g + i, carry)
            store_group(jnp.maximum(g - 2, 0), (i,))
            load_group(jnp.minimum(g + 2, NG - 1), (i,))
        return carry

    init = (_dup(mem0_ref[...].astype(F32)), jnp.zeros((SEG, DP), F32),
            jnp.full((8, 128), -jnp.inf, F32), jnp.zeros((8, 128), jnp.int32))
    _, attn, best, arg = lax.fori_loop(0, NG, group, init)
    for cp in cp_ffn:
        cp.wait()
    best, arg = post(NSEG - 1, attn, True, best, arg)

    top = jnp.max(best, axis=0, keepdims=True)
    idx = jnp.min(jnp.where(best == top, arg, S - 1))
    idx = jnp.clip(idx, 0, S - 1)
    xsel = jnp.concatenate([h2_s[t, pl.ds(idx, 1), :] for t in range(4)], axis=1)
    xsel = jnp.broadcast_to(xsel, (8, DP))[:, 0:D]
    store_group(NG - 2)
    store_group(NG - 1)
    gate = jnp.dot(xsel, wg_v[...], preferred_element_type=F32)
    up = jnp.dot(xsel, wu_v[...], preferred_element_type=F32)
    for g in range(NG - 3, NG):
        out_copy(g).start()
    act = gate * jax.nn.sigmoid(gate) * up
    y = lax.dot_general(act, wd_v[...], NT, preferred_element_type=F32)
    y = _dup(y) * jax.nn.sigmoid(top[:, 0:1]) * vec_s[5]
    for t in range(4):
        o_s[t, pl.ds(idx, 1), :] = o_s[t, pl.ds(idx, 1), :] + y[0:1, 128 * t:128 * t + 128]
    for g in range(NG):
        out_copy(g).wait()
    store_group(idx // 128)
    patch = out_copy(idx // 128)
    patch.start()
    patch.wait()


@functools.partial(jax.jit, static_argnames=("A_seg_len",))
def pallas_adaLN_cond__memory_aug_recurrent_mem_tr__moe_arch_mod__prompt_kernel(
        A_x, A_mem0, A_Wq, A_Wk, A_Wv, A_Wo, A_seg_len, B_x, B_w_r, B_w_gate, B_w_up, B_w_down, c, w_mod):
    del B_x
    assert A_seg_len == SEG and A_x.shape == (1, S, D) and A_Wq.shape == (D, H, E)
    hbm = pl.BlockSpec(memory_space=pl.ANY)
    outT = pl.pallas_call(
        _kernel,
        out_shape=jax.ShapeDtypeStruct((D, S), A_x.dtype),
        in_specs=[hbm] * 12,
        out_specs=hbm,
        scratch_shapes=[
            pltpu.VMEM((M, D), BF16),
            pltpu.VMEM((D,), BF16),
            pltpu.VMEM((1, D), BF16),
            pltpu.VMEM((2, D * H, 128), BF16),
            pltpu.VMEM((2, D * H, 128), BF16),
            pltpu.VMEM((2, D * H, 128), BF16),
            pltpu.VMEM((2, H, D, 128), BF16),
            pltpu.VMEM((H, 3, D, 128), F32),
            pltpu.VMEM((H // 2, 128, DP), F32),
            pltpu.VMEM((D, 6 * D), BF16),
            pltpu.VMEM((D, FF), BF16),
            pltpu.VMEM((D, FF), BF16),
            pltpu.VMEM((D, FF), BF16),
            pltpu.VMEM((NG, DP, 128), BF16),
            pltpu.VMEM((192, NW), U32),
            pltpu.VMEM((DP // 2, 64 * H), U32),
            pltpu.VMEM((192, NW), U32),
            pltpu.VMEM((32 * H, DP), U32),
            pltpu.VMEM((7, 8, DP), F32),
            pltpu.VMEM((4, S, 128), F32),
            pltpu.VMEM((4, S + SEG, 128), F32),
            pltpu.VMEM((4, S + SEG, 128), F32),
            pltpu.VMEM((NG, DP, 128), BF16),
            pltpu.SemaphoreType.DMA((NSEM,)),
            pltpu.SemaphoreType.DMA((1,)),
        ],
        compiler_params=pltpu.CompilerParams(vmem_limit_bytes=100 * 1024 * 1024),
        name="adaln_rmt_mod",
    )(
        A_x.reshape(S, D).T,
        A_mem0.reshape(M, D),
        A_Wq.reshape(D * H, E),
        A_Wk.reshape(D * H, E),
        A_Wv.reshape(D * H, E),
        A_Wo.transpose(0, 2, 1),
        B_w_r,
        B_w_gate,
        B_w_up,
        B_w_down.T,
        c,
        w_mod,
    )
    return outT.T.reshape(1, S, D)
```

```python
import functools

import jax
import jax.numpy as jnp
from jax import lax
from jax.experimental import pallas as pl
from jax.experimental.pallas import tpu as pltpu

F32 = jnp.float32
BF16 = jnp.bfloat16
U32 = jnp.uint32

S, D, H, E, M, SEG, FF = 2048, 448, 16, 256, 8, 32, 1792
DP = 512
NSEG = S // SEG
NG = S // 128
L = SEG + M
NW = H * D
NT = (((1,), (1,)), ((), ()))
EPS = 1e-5
NSEM = 21

ORDER = ("Q K316 T2 K02 T0 K02 K04 T1 S31 T3 S34 S30 K04 K04 K14 T4 T5 S32 T6 T7 K14 K14 K14 "
         "S04 S00 S01 S02 K22 K22 K24 S03 S13 S11 S14 K22 K22 K24 S10 S33 S12 V38 V38 S24 V04 "
         "S20 S21 S22 S23 X V02 V02 V04 V14 V04 V14 V14 V24 V14 V24 V24 V24 U0 U1 U3 U7 U2 U4 U6 U5").split()


def _dup(v):
    return jnp.concatenate([v, v[:, 384:448]], axis=1)


def _rowsum(v):
    t = v[:, 0:128] + v[:, 128:256] + v[:, 256:384] + 0.5 * v[:, 384:512]
    return jnp.sum(t, axis=1, keepdims=True)


def _layernorm(v):
    mu = _rowsum(v) * (1.0 / D)
    d = v - mu
    var = _rowsum(d * d) * (1.0 / D)
    return d * lax.rsqrt(var + EPS)


def _group8(v, op, lane):
    for d in (1, 2, 4):
        up = pltpu.roll(v, d, 1)
        dn = pltpu.roll(v, 128 - d, 1)
        v = op(v, jnp.where((lane & d) != 0, up, dn))
    return v


def _unpack(u):
    lo = pltpu.bitcast(u << 16, F32)
    hi = pltpu.bitcast(u & jnp.uint32(0xFFFF0000), F32)
    return lo, hi


def _kernel(xT_hbm, mem0_hbm, wq_hbm, wk_hbm, wv_hbm, woT_hbm, wr_hbm, wg_hbm, wu_hbm, wdT_hbm,
            c_hbm, wmod_hbm, out_hbm,
            mem0_ref, wr_ref, c_ref, wq_v, wk_v, wv_v, wo_v, acc_s, acct_s, wmod_v, wg_v, wu_v, wd_v, xs_v,
            wk1_s, wq2_s, wv1_s, wb2_s, vec_s, x_s, o_s, h2_s, st_s, sems, osem):
    sem_ids = iter(range(NSEM))

    def copy(src, dst):
        return pltpu.make_async_copy(src, dst, sems.at[next(sem_ids)])

    def slab(col):
        return pl.ds(pl.multiple_of(col, 128), 128)

    def x_group(g, k):
        cols = pl.ds(128 * g, 128)
        return [pltpu.make_async_copy(xT_hbm.at[:, cols], xs_v.at[g, pl.ds(0, D)], sems.at[k]),
                pltpu.make_async_copy(xT_hbm.at[pl.ds(384, 64), cols], xs_v.at[g, pl.ds(D, 64)], sems.at[k])]

    def rows_copy(src, dst, e, d0, n):
        return copy(src.at[pl.ds(H * d0, H * n), pl.ds(128 * e, 128)], dst.at[e, pl.ds(H * d0, H * n)])

    cp_qk = [[[rows_copy(wk_hbm, wk_v, e, 0, D), rows_copy(wq_hbm, wq_v, e, 0, 256)],
              [rows_copy(wq_hbm, wq_v, e, 256, D - 256)]] for e in range(2)]

    def wo_copy(e, a):
        hs = pl.ds(8 * a, 8)
        return copy(woT_hbm.at[hs, :, pl.ds(128 * e, 128)], wo_v.at[e, hs])

    cp_vo = [[[rows_copy(wv_hbm, wv_v, e, 0, D), wo_copy(e, 0)], [wo_copy(e, 1)]] for e in range(2)]
    k_x0, k_x = next(sem_ids), next(sem_ids)
    cp_x0 = [cp for g in range(3) for cp in x_group(g, k_x0)]
    cp_mod = [copy(c_hbm, c_ref), copy(wr_hbm, wr_ref), copy(mem0_hbm, mem0_ref), copy(wmod_hbm, wmod_v)]
    cp_x = [cp for g in range(3, NG) for cp in x_group(g, k_x)]
    cp_ffn = [copy(wg_hbm, wg_v), copy(wu_hbm, wu_v), copy(wdT_hbm, wd_v)]
    for cp in sum(sum(cp_qk + cp_vo, []), []) + cp_x0 + cp_mod + cp_x + cp_ffn:
        cp.start()

    lane = lax.broadcasted_iota(jnp.int32, (8, 128), 1)
    sub = lax.broadcasted_iota(jnp.int32, (8, 128), 0)
    low = lane < 64
    low64 = lax.broadcasted_iota(jnp.int32, (64, 128), 1) < 64

    def pair_rows(buf, e, p, d0, n):
        view = buf.bitcast(U32).at[e, pl.ds(8 * d0, 8 * n)]
        return _unpack(view[pl.ds(p, n, stride=8), :])

    def packed(r):
        return pltpu.bitcast(r.astype(BF16), U32)

    def fold_main(lhs, rhs, e, t, p, dst, scale):
        rest = []
        for i in range(2):
            r = lax.dot_general(lhs[i], rhs[i].astype(BF16), NT, preferred_element_type=F32)
            if e == 0:
                acc_s[2 * p + i, t] = r
                continue
            r = (r + acc_s[2 * p + i, t]) * scale
            c0 = t * 2048 + (2 * p + i) * 128
            dst[:, c0:c0 + 128] = packed(r[0:384])
            rest.append(r[384:448])
        return jnp.concatenate(rest, axis=0) if e else None

    def fold_tail(lhs, rhs, e, p, dst, scale):
        both = jnp.concatenate([lhs[0][384:448], lhs[1][384:448]], axis=0)
        r = jnp.concatenate(
            [lax.dot_general(rhs[i], jnp.concatenate([lhs[i][0:384], both], axis=0).astype(BF16), NT,
                             preferred_element_type=F32) for i in range(2)], axis=0)
        if e == 0:
            acct_s[p] = r
            return None
        r = (r + acct_s[p]) * scale
        dst[:, 3 * 2048 + p * 128:3 * 2048 + p * 128 + 128] = packed(r[:, 0:384].T)
        return r[:, 384:512]

    def fold_qk(e, part, p):
        k = pair_rows(wk_v, e, p, 0, D)
        for t in ((0, 1), (2,))[part]:
            rest = fold_main(k, pair_rows(wq_v, e, p, 128 * t, 128), e, t, p, wk1_s, E ** -0.5)
            if e:
                wq2_s[64 * t:64 * t + 64, 128 * p:128 * p + 128] = packed(rest.T)
        if part:
            r = fold_tail(k, pair_rows(wq_v, e, p, 384, 64), e, p, wk1_s, E ** -0.5)
            if e:
                r = jnp.concatenate([jnp.where(low64, r[0:64], r[64:128]), jnp.zeros((64, 128), F32)], axis=0)
                wq2_s[192:256, 128 * p:128 * p + 128] = packed(r)

    def fold_vo(e, p):
        v = pair_rows(wv_v, e, p, 0, D)
        for t in range(3):
            rest = fold_main(v, [wo_v[e, 2 * p + i, 128 * t:128 * t + 128, :] for i in range(2)],
                             e, t, p, wv1_s, 1.0)
            if e:
                wb2_s[64 * p:64 * p + 64, 128 * t:128 * t + 128] = packed(rest)
        r = fold_tail(v, [wo_v[e, 2 * p + i, 384:448, :].astype(F32) for i in range(2)], e, p, wv1_s, 1.0)
        if e:
            r = r.T
            o = pltpu.roll(r, 64, 1)
            wb2_s[64 * p:64 * p + 64, 384:512] = packed(jnp.concatenate(
                [jnp.where(low64, r[0:64], o[0:64]), jnp.where(low64, o[64:128], r[64:128])], axis=0))

    for e in range(2):
        for part in range(2):
            for cp in cp_qk[e][part]:
                cp.wait()
            for p in range(H // 2):
                fold_qk(e, part, p)
    for e in range(2):
        for a in range(2):
            for cp in cp_vo[e][a]:
                cp.wait()
            for p in range(4 * a, 4 * a + 4):
                fold_vo(e, p)

    for cp in cp_x0 + cp_mod:
        cp.wait()
    cv = jnp.broadcast_to(c_ref[...].astype(F32), (8, D))
    mod = jnp.dot(cv * jax.nn.sigmoid(cv), wmod_v[...], preferred_element_type=F32)
    for k in range(6):
        m = _dup(mod[:, D * k:D * (k + 1)])
        vec_s[k] = 1.0 + m if k in (1, 4) else m
    vec_s[6] = _dup(jnp.broadcast_to(wr_ref[...].astype(F32).reshape(1, D), (8, D)))

    def vec(k):
        return jnp.concatenate([vec_s[k]] * (SEG // 8), axis=0)

    def rows_of(g):
        return pl.ds(pl.multiple_of(g * 128, 128), 128)

    def load_group(g, ts=range(4)):
        for t in ts:
            x_s[t, rows_of(g), :] = xs_v[g, 128 * t:128 * t + 128, :].astype(F32).T

    def store_group(g, ts=range(4)):
        for t in ts:
            st_s[g, 128 * t:128 * t + 128, :] = o_s[t, rows_of(g), :].T.astype(BF16)

    def seg_rows(ref, s):
        r0 = pl.multiple_of(s * SEG, SEG)
        return jnp.concatenate([ref[t, pl.ds(r0, SEG), :] for t in range(4)], axis=1)

    def pre(s):
        h = _layernorm(seg_rows(x_s, s)) * vec(1) + vec(0)
        for t in range(4):
            (o_s, h2_s)[t // 2][t % 2, S:S + SEG, :] = h[:, 128 * t:128 * t + 128]

    def parked():
        return jnp.concatenate([(o_s, h2_s)[t // 2][t % 2, S:S + SEG, :] for t in range(4)], axis=1)

    def post(s, attn, valid, best, arg):
        x1 = seg_rows(x_s, s) + vec(2) * attn
        h2 = _layernorm(x1) * vec(4) + vec(3)
        out = x1 + vec(5) * h2
        r = _rowsum(h2 * vec(6))
        r0 = pl.multiple_of(s * SEG, SEG)
        for t in range(4):
            o_s[t, pl.ds(r0, SEG), :] = out[:, 128 * t:128 * t + 128]
            h2_s[t, pl.ds(r0, SEG), :] = h2[:, 128 * t:128 * t + 128]
        for g in range(SEG // 8):
            rg = jnp.broadcast_to(r[8 * g:8 * g + 8], (8, 128))
            upd = jnp.logical_and(rg > best, valid)
            best = jnp.where(upd, rg, best)
            arg = jnp.where(upd, s * SEG + 8 * g + sub, arg)
        return best, arg

    def project(h1, w_ref, t, h0, hn, dup):
        w = 128 if t < 3 else 64
        c0 = 2048 * t + w * h0
        r = jnp.dot(h1, pltpu.bitcast(w_ref[:, c0:c0 + w * (hn - h0)], BF16), preferred_element_type=F32)
        tiles = []
        for j in range(L // 8):
            rows = r[8 * j:8 * j + 8]
            if t < 3:
                parts = [rows[:, 128 * h:128 * h + 128] for h in range(hn - h0)]
            else:
                parts = []
                for p in range((hn - h0) // 2):
                    v = rows[:, 128 * p:128 * p + 128]
                    o = pltpu.roll(v, 64, 1) if dup else 0.0
                    parts += [jnp.where(low, v, o), jnp.where(low, o, v)]
            tiles.append(jnp.concatenate(parts, axis=0))
        return tiles

    def barrel(src, want):
        def stage(k, c):
            if k < 0:
                return src[c]
            key = (k, c)
            if key not in memo:
                hi, lo = stage(k - 1, (c + (1 << k)) % 8), stage(k - 1, c)
                memo[key] = lo if hi is None else hi if lo is None else jnp.where((lane & (16 << k)) != 0, hi, lo)
            return memo[key]
        memo = {}
        return [stage(2, c) for c in want]

    def softmax(sc, tt):
        p_rows, z_rows = [], []
        for g in (4, 0, 1, 2, 3):
            extra = barrel([t[8 * g:8 * g + 8] for t in tt], [(-j) % 8 for j in range(L // 8)])
            blk = []
            for j in range(L // 8):
                if g < j < 4:
                    blk.append(jnp.full((8, 128), -1e9, F32))
                    continue
                r0 = 8 * (g - j) if j < SEG // 8 else 8 * g
                v = sc[j][r0:r0 + 8] + (pltpu.roll(extra[j], 128 - 16 * j, 1) if j else extra[j])
                if g < 4 and j == g:
                    v = jnp.where((lane & 7) <= sub, v, -1e9)
                blk.append(v)
            m = _group8(functools.reduce(jnp.maximum, blk), jnp.maximum, lane)
            ex = [jnp.exp(v - m) for v in blk]
            inv = 1.0 / _group8(functools.reduce(jnp.add, ex), jnp.add, lane)
            pr = [e * inv for e in ex]
            p_rows.append(jnp.concatenate(pr, axis=1))
            rolled = [pltpu.roll(v, 16 * j, 1) if j else v for j, v in enumerate(pr)]
            z_rows.append(jnp.concatenate(barrel(rolled + [None] * 3, [(-i) % 8 for i in range(8)]), axis=1))
        return jnp.concatenate(p_rows, axis=0), jnp.concatenate(z_rows, axis=0)

    load_group(0)
    load_group(1)
    pre(0)
    for t in range(4):
        o_s[t, 0:128, :] = jnp.zeros((128, 128), F32)

    def out_copy(g):
        return pltpu.make_async_copy(st_s.at[g, pl.ds(0, D)], out_hbm.at[:, slab(g * 128)], osem.at[0])

    def step(s, carry):
        mem, attn, best, arg = carry
        hh = jnp.concatenate([parked(), mem], axis=0)
        h1 = hh[:, 0:384]
        best, arg = post(jnp.maximum(s - 1, 0), attn, s > 0, best, arg)
        pre(jnp.minimum(s + 1, NSEG - 1))

        tails = []
        for j in range(L // 8):
            v = hh[8 * j:8 * j + 8, 384:512]
            tails.append(jnp.concatenate([jnp.where(low, v, 0.0), jnp.where(low, 0.0, v)], axis=0))
        tails += [jnp.zeros((16, 128), F32)] * 3
        tail_rhs = [jnp.concatenate([tails[(b - i) % 8] for b in range(8)], axis=0).astype(BF16)
                    for i in range(8)]

        sc = [None] * (L // 8)
        kp = {t: [] for t in range(4)}
        vt = {t: [] for t in range(4)}
        kd, vd, tl, ul = {}, {}, {}, {}
        for op in ORDER:
            if op[0] == 'Q':
                q2 = jnp.dot(hh, pltpu.bitcast(wq2_s[...], BF16), preferred_element_type=F32)
            elif op[0] == 'K':
                t, n = int(op[1]), int(op[2:])
                h0 = kd.get(t, 0)
                kp[t].append(project(h1, wk1_s, t, h0, h0 + n, False))
                kd[t] = h0 + n
            elif op[0] == 'V':
                t, n = int(op[1]), int(op[2:])
                h0 = vd.get(t, 0)
                vt[t].append(project(h1, wv1_s, t, h0, h0 + n, True))
                vd[t] = h0 + n
            elif op[0] == 'T':
                i = int(op[1])
                tl[i] = lax.dot_general(q2[:, 128 * i:128 * i + 128], tail_rhs[i], NT, preferred_element_type=F32)
            elif op[0] == 'S':
                t, j = int(op[1]), int(op[2])
                kt = jnp.concatenate([piece[j] for piece in kp[t]], axis=0)
                r0 = 8 * j if j < SEG // 8 else 0
                d = lax.dot_general(hh[r0:, 128 * t:128 * t + 128], kt.astype(BF16), NT, preferred_element_type=F32)
                sc[j] = d if sc[j] is None else sc[j] + d
            elif op[0] == 'X':
                p, z = softmax(sc, [tl[i] for i in range(8)])
            elif op[0] == 'U':
                i = int(op[1])
                ul[i] = jnp.dot(z[:, 128 * i:128 * i + 128], tail_rhs[i], preferred_element_type=F32)
        u = jnp.concatenate([ul[i] for i in range(8)], axis=1)
        vmat = jnp.concatenate(
            [jnp.concatenate([piece[j] for j in range(L // 8) for piece in vt[t]], axis=0) for t in range(4)],
            axis=1)
        o = jnp.dot(p, vmat.astype(BF16), preferred_element_type=F32)
        o = jnp.dot(u, pltpu.bitcast(wb2_s[...], BF16), preferred_element_type=F32) + o
        return o[0:M], o[M:L], best, arg

    def group(g, carry):
        for i in range(4):
            carry = step(4 * g + i, carry)
            store_group(jnp.maximum(g - 2, 0), (i,))
            load_group(jnp.minimum(g + 2, NG - 1), (i,))

        @pl.when(g == 0)
        def _():
            for cp in cp_x:
                cp.wait()

        @pl.when(g >= 2)
        def _():
            out_copy(g - 2).start()

        return carry

    init = (_dup(mem0_ref[...].astype(F32)), jnp.zeros((SEG, DP), F32),
            jnp.full((8, 128), -jnp.inf, F32), jnp.zeros((8, 128), jnp.int32))
    _, attn, best, arg = lax.fori_loop(0, NG, group, init)
    for cp in cp_ffn:
        cp.wait()
    best, arg = post(NSEG - 1, attn, True, best, arg)

    top = jnp.max(best, axis=0, keepdims=True)
    idx = jnp.min(jnp.where(best == top, arg, S - 1))
    idx = jnp.clip(idx, 0, S - 1)
    xsel = jnp.concatenate([h2_s[t, pl.ds(idx, 1), :] for t in range(4)], axis=1)
    xsel = jnp.broadcast_to(xsel, (8, DP))[:, 0:D]
    store_group(NG - 2)
    store_group(NG - 1)
    gate = jnp.dot(xsel, wg_v[...], preferred_element_type=F32)
    up = jnp.dot(xsel, wu_v[...], preferred_element_type=F32)
    for g in range(NG - 2, NG):
        out_copy(g).start()
    act = gate * jax.nn.sigmoid(gate) * up
    y = lax.dot_general(act, wd_v[...], NT, preferred_element_type=F32)
    y = _dup(y) * jax.nn.sigmoid(top[:, 0:1]) * vec_s[5]
    for t in range(4):
        o_s[t, pl.ds(idx, 1), :] = o_s[t, pl.ds(idx, 1), :] + y[0:1, 128 * t:128 * t + 128]
    for g in range(NG):
        out_copy(g).wait()
    store_group(idx // 128)
    patch = out_copy(idx // 128)
    patch.start()
    patch.wait()


@functools.partial(jax.jit, static_argnames=("A_seg_len",))
def pallas_adaLN_cond__memory_aug_recurrent_mem_tr__moe_arch_mod__prompt_kernel(
        A_x, A_mem0, A_Wq, A_Wk, A_Wv, A_Wo, A_seg_len, B_x, B_w_r, B_w_gate, B_w_up, B_w_down, c, w_mod):
    del B_x
    assert A_seg_len == SEG and A_x.shape == (1, S, D) and A_Wq.shape == (D, H, E)
    hbm = pl.BlockSpec(memory_space=pl.ANY)
    outT = pl.pallas_call(
        _kernel,
        out_shape=jax.ShapeDtypeStruct((D, S), A_x.dtype),
        in_specs=[hbm] * 12,
        out_specs=hbm,
        scratch_shapes=[
            pltpu.VMEM((M, D), BF16),
            pltpu.VMEM((D,), BF16),
            pltpu.VMEM((1, D), BF16),
            pltpu.VMEM((2, D * H, 128), BF16),
            pltpu.VMEM((2, D * H, 128), BF16),
            pltpu.VMEM((2, D * H, 128), BF16),
            pltpu.VMEM((2, H, D, 128), BF16),
            pltpu.VMEM((H, 3, D, 128), F32),
            pltpu.VMEM((H // 2, 128, DP), F32),
            pltpu.VMEM((D, 6 * D), BF16),
            pltpu.VMEM((D, FF), BF16),
            pltpu.VMEM((D, FF), BF16),
            pltpu.VMEM((D, FF), BF16),
            pltpu.VMEM((NG, DP, 128), BF16),
            pltpu.VMEM((192, NW), U32),
            pltpu.VMEM((DP // 2, 64 * H), U32),
            pltpu.VMEM((192, NW), U32),
            pltpu.VMEM((32 * H, DP), U32),
            pltpu.VMEM((7, 8, DP), F32),
            pltpu.VMEM((4, S, 128), F32),
            pltpu.VMEM((4, S + SEG, 128), F32),
            pltpu.VMEM((4, S + SEG, 128), F32),
            pltpu.VMEM((NG, DP, 128), BF16),
            pltpu.SemaphoreType.DMA((NSEM,)),
            pltpu.SemaphoreType.DMA((1,)),
        ],
        compiler_params=pltpu.CompilerParams(vmem_limit_bytes=100 * 1024 * 1024),
        name="adaln_rmt_mod",
    )(
        A_x.reshape(S, D).T,
        A_mem0.reshape(M, D),
        A_Wq.reshape(D * H, E),
        A_Wk.reshape(D * H, E),
        A_Wv.reshape(D * H, E),
        A_Wo.transpose(0, 2, 1),
        B_w_r,
        B_w_gate,
        B_w_up,
        B_w_down.T,
        c,
        w_mod,
    )
    return outT.T.reshape(1, S, D)
```

```python
import functools

import jax
import jax.numpy as jnp
from jax import lax
from jax.experimental import pallas as pl
from jax.experimental.pallas import tpu as pltpu

F32 = jnp.float32
BF16 = jnp.bfloat16
U32 = jnp.uint32

S, D, H, E, M, SEG, FF = 2048, 448, 16, 256, 8, 32, 1792
DP = 512
NSEG = S // SEG
NG = S // 128
L = SEG + M
NW = H * D
NT = (((1,), (1,)), ((), ()))
EPS = 1e-5
NSEM = 21

ORDER = ("B Q K316 A T2 K02 T0 K02 K04 C T1 S31 S34 T3 S30 K04 K04 K14 T4 T5 S32 T6 T7 K14 K14 K14 S04 S01 "
         "S02 S00 K22 K22 K22 K22 S03 S13 S11 S14 K24 K22 K22 S10 S33 S12 V316 S24 V04 S20 S21 S22 S23 X "
         "V02 V04 V02 V02 V14 D V18 V02 V24 V14 V212 U0 U3 U7 U2 U4 U6 U5 U1").split()


def _dup(v):
    return jnp.concatenate([v, v[:, 384:448]], axis=1)


def _rowsum(v):
    t = v[:, 0:128] + v[:, 128:256] + v[:, 256:384] + 0.5 * v[:, 384:512]
    return jnp.sum(t, axis=1, keepdims=True)


def _layernorm(v):
    mu = _rowsum(v) * (1.0 / D)
    d = v - mu
    var = _rowsum(d * d) * (1.0 / D)
    return d * lax.rsqrt(var + EPS)


def _group8(v, op, lane):
    for d in (1, 2, 4):
        up = pltpu.roll(v, d, 1)
        dn = pltpu.roll(v, 128 - d, 1)
        v = op(v, jnp.where((lane & d) != 0, up, dn))
    return v


def _unpack(u):
    lo = pltpu.bitcast(u << 16, F32)
    hi = pltpu.bitcast(u & jnp.uint32(0xFFFF0000), F32)
    return lo, hi


def _kernel(xT_hbm, mem0_hbm, wq_hbm, wk_hbm, wv_hbm, woT_hbm, wr_hbm, wg_hbm, wu_hbm, wdT_hbm,
            c_hbm, wmod_hbm, out_hbm,
            mem0_ref, wr_ref, c_ref, wq_v, wk_v, wv_v, wo_v, acc_s, acct_s, wmod_v, wg_v, wu_v, wd_v, xs_v,
            wk1_s, wq2_s, wv1_s, wb2_s, vec_s, x_s, o_s, h2_s, st_s, sems, osem):
    sem_ids = iter(range(NSEM))

    def copy(src, dst):
        return pltpu.make_async_copy(src, dst, sems.at[next(sem_ids)])

    def slab(col):
        return pl.ds(pl.multiple_of(col, 128), 128)

    def x_group(g, k):
        cols = pl.ds(128 * g, 128)
        return [pltpu.make_async_copy(xT_hbm.at[:, cols], xs_v.at[g, pl.ds(0, D)], sems.at[k]),
                pltpu.make_async_copy(xT_hbm.at[pl.ds(384, 64), cols], xs_v.at[g, pl.ds(D, 64)], sems.at[k])]

    def rows_copy(src, dst, e, d0, n):
        return copy(src.at[pl.ds(H * d0, H * n), pl.ds(128 * e, 128)], dst.at[e, pl.ds(H * d0, H * n)])

    cp_qk = [[[rows_copy(wk_hbm, wk_v, e, 0, D), rows_copy(wq_hbm, wq_v, e, 0, 256)],
              [rows_copy(wq_hbm, wq_v, e, 256, D - 256)]] for e in range(2)]

    def wo_copy(e, a):
        hs = pl.ds(8 * a, 8)
        return copy(woT_hbm.at[hs, :, pl.ds(128 * e, 128)], wo_v.at[e, hs])

    cp_vo = [[[rows_copy(wv_hbm, wv_v, e, 0, D), wo_copy(e, 0)], [wo_copy(e, 1)]] for e in range(2)]
    k_x0, k_x = next(sem_ids), next(sem_ids)
    cp_x0 = [cp for g in range(3) for cp in x_group(g, k_x0)]
    cp_mod = [copy(c_hbm, c_ref), copy(wr_hbm, wr_ref), copy(mem0_hbm, mem0_ref), copy(wmod_hbm, wmod_v)]
    cp_x = [cp for g in range(3, NG) for cp in x_group(g, k_x)]
    cp_ffn = [copy(wg_hbm, wg_v), copy(wu_hbm, wu_v), copy(wdT_hbm, wd_v)]
    for cp in sum(sum(cp_qk + cp_vo, []), []) + cp_x0 + cp_mod + cp_x + cp_ffn:
        cp.start()

    lane = lax.broadcasted_iota(jnp.int32, (8, 128), 1)
    sub = lax.broadcasted_iota(jnp.int32, (8, 128), 0)
    low = lane < 64
    low64 = lax.broadcasted_iota(jnp.int32, (64, 128), 1) < 64

    def pair_rows(buf, e, p, d0, n):
        view = buf.bitcast(U32).at[e, pl.ds(8 * d0, 8 * n)]
        return _unpack(view[pl.ds(p, n, stride=8), :])

    def packed(r):
        return pltpu.bitcast(r.astype(BF16), U32)

    def fold_main(lhs, rhs, e, t, p, dst, scale):
        rest = []
        for i in range(2):
            r = lax.dot_general(lhs[i], rhs[i].astype(BF16), NT, preferred_element_type=F32)
            if e == 0:
                acc_s[2 * p + i, t] = r
                continue
            r = (r + acc_s[2 * p + i, t]) * scale
            c0 = t * 2048 + (2 * p + i) * 128
            dst[:, c0:c0 + 128] = packed(r[0:384])
            rest.append(r[384:448])
        return jnp.concatenate(rest, axis=0) if e else None

    def fold_tail(lhs, rhs, e, p, dst, scale):
        both = jnp.concatenate([lhs[0][384:448], lhs[1][384:448]], axis=0)
        r = jnp.concatenate(
            [lax.dot_general(rhs[i], jnp.concatenate([lhs[i][0:384], both], axis=0).astype(BF16), NT,
                             preferred_element_type=F32) for i in range(2)], axis=0)
        if e == 0:
            acct_s[p] = r
            return None
        r = (r + acct_s[p]) * scale
        dst[:, 3 * 2048 + p * 128:3 * 2048 + p * 128 + 128] = packed(r[:, 0:384].T)
        return r[:, 384:512]

    def fold_qk(e, part, p):
        k = pair_rows(wk_v, e, p, 0, D)
        for t in ((0, 1), (2,))[part]:
            rest = fold_main(k, pair_rows(wq_v, e, p, 128 * t, 128), e, t, p, wk1_s, E ** -0.5)
            if e:
                wq2_s[64 * t:64 * t + 64, 128 * p:128 * p + 128] = packed(rest.T)
        if part:
            r = fold_tail(k, pair_rows(wq_v, e, p, 384, 64), e, p, wk1_s, E ** -0.5)
            if e:
                r = jnp.concatenate([jnp.where(low64, r[0:64], r[64:128]), jnp.zeros((64, 128), F32)], axis=0)
                wq2_s[192:256, 128 * p:128 * p + 128] = packed(r)

    def fold_vo(e, p):
        v = pair_rows(wv_v, e, p, 0, D)
        for t in range(3):
            rest = fold_main(v, [wo_v[e, 2 * p + i, 128 * t:128 * t + 128, :] for i in range(2)],
                             e, t, p, wv1_s, 1.0)
            if e:
                wb2_s[64 * p:64 * p + 64, 128 * t:128 * t + 128] = packed(rest)
        r = fold_tail(v, [wo_v[e, 2 * p + i, 384:448, :].astype(F32) for i in range(2)], e, p, wv1_s, 1.0)
        if e:
            r = r.T
            o = pltpu.roll(r, 64, 1)
            wb2_s[64 * p:64 * p + 64, 384:512] = packed(jnp.concatenate(
                [jnp.where(low64, r[0:64], o[0:64]), jnp.where(low64, o[64:128], r[64:128])], axis=0))

    for e in range(2):
        for part in range(2):
            for cp in cp_qk[e][part]:
                cp.wait()
            for p in range(H // 2):
                fold_qk(e, part, p)
    for e in range(2):
        for a in range(2):
            for cp in cp_vo[e][a]:
                cp.wait()
            for p in range(4 * a, 4 * a + 4):
                fold_vo(e, p)

    for cp in cp_x0 + cp_mod:
        cp.wait()
    cv = jnp.broadcast_to(c_ref[...].astype(F32), (8, D))
    mod = jnp.dot(cv * jax.nn.sigmoid(cv), wmod_v[...], preferred_element_type=F32)
    for k in range(6):
        m = _dup(mod[:, D * k:D * (k + 1)])
        vec_s[k] = 1.0 + m if k in (1, 4) else m
    vec_s[6] = _dup(jnp.broadcast_to(wr_ref[...].astype(F32).reshape(1, D), (8, D)))

    def vec(k):
        return jnp.concatenate([vec_s[k]] * (SEG // 8), axis=0)

    def rows_of(g):
        return pl.ds(pl.multiple_of(g * 128, 128), 128)

    def load_group(g, ts=range(4)):
        for t in ts:
            x_s[t, rows_of(g), :] = xs_v[g, 128 * t:128 * t + 128, :].astype(F32).T

    def store_group(g, ts=range(4)):
        for t in ts:
            st_s[g, 128 * t:128 * t + 128, :] = o_s[t, rows_of(g), :].T.astype(BF16)

    def seg_rows(ref, s):
        r0 = pl.multiple_of(s * SEG, SEG)
        return jnp.concatenate([ref[t, pl.ds(r0, SEG), :] for t in range(4)], axis=1)

    def pre(s):
        h = _layernorm(seg_rows(x_s, s)) * vec(1) + vec(0)
        for t in range(4):
            (o_s, h2_s)[t // 2][t % 2, S:S + SEG, :] = h[:, 128 * t:128 * t + 128]

    def parked():
        return jnp.concatenate([(o_s, h2_s)[t // 2][t % 2, S:S + SEG, :] for t in range(4)], axis=1)

    def post(s, attn, valid, best, arg):
        x1 = seg_rows(x_s, s) + vec(2) * attn
        h2 = _layernorm(x1) * vec(4) + vec(3)
        out = x1 + vec(5) * h2
        r = _rowsum(h2 * vec(6))
        r0 = pl.multiple_of(s * SEG, SEG)
        for t in range(4):
            o_s[t, pl.ds(r0, SEG), :] = out[:, 128 * t:128 * t + 128]
            h2_s[t, pl.ds(r0, SEG), :] = h2[:, 128 * t:128 * t + 128]
        for g in range(SEG // 8):
            rg = jnp.broadcast_to(r[8 * g:8 * g + 8], (8, 128))
            upd = jnp.logical_and(rg > best, valid)
            best = jnp.where(upd, rg, best)
            arg = jnp.where(upd, s * SEG + 8 * g + sub, arg)
        return best, arg

    def project(h1, w_ref, t, h0, hn):
        w = 128 if t < 3 else 64
        c0 = 2048 * t + w * h0
        r = jnp.dot(h1, pltpu.bitcast(w_ref[:, c0:c0 + w * (hn - h0)], BF16), preferred_element_type=F32)
        tiles = []
        for j in range(L // 8):
            rows = r[8 * j:8 * j + 8]
            if t < 3:
                parts = [rows[:, 128 * h:128 * h + 128] for h in range(hn - h0)]
            else:
                parts = []
                for p in range((hn - h0) // 2):
                    v = rows[:, 128 * p:128 * p + 128]
                    parts += [jnp.where(low, v, 0.0), jnp.where(low, 0.0, v)]
            tiles.append(jnp.concatenate(parts, axis=0))
        return tiles

    def barrel(src, want):
        def stage(k, c):
            if k < 0:
                return src[c]
            key = (k, c)
            if key not in memo:
                hi, lo = stage(k - 1, (c + (1 << k)) % 8), stage(k - 1, c)
                memo[key] = lo if hi is None else hi if lo is None else jnp.where((lane & (16 << k)) != 0, hi, lo)
            return memo[key]
        memo = {}
        return [stage(2, c) for c in want]

    def softmax(sc, tt):
        p_rows, z_rows = [], []
        for g in (4, 0, 1, 2, 3):
            extra = barrel([t[8 * g:8 * g + 8] for t in tt], [(-j) % 8 for j in range(L // 8)])
            blk = []
            for j in range(L // 8):
                if g < j < 4:
                    blk.append(jnp.full((8, 128), -1e9, F32))
                    continue
                r0 = 8 * (g - j) if j < SEG // 8 else 8 * g
                v = sc[j][r0:r0 + 8] + (pltpu.roll(extra[j], 128 - 16 * j, 1) if j else extra[j])
                if g < 4 and j == g:
                    v = jnp.where((lane & 7) <= sub, v, -1e9)
                blk.append(v)
            m = _group8(functools.reduce(jnp.maximum, blk), jnp.maximum, lane)
            ex = [jnp.exp(v - m) for v in blk]
            inv = 1.0 / _group8(functools.reduce(jnp.add, ex), jnp.add, lane)
            pr = [e * inv for e in ex]
            p_rows.append(jnp.concatenate(pr, axis=1))
            rolled = [pltpu.roll(v, 16 * j, 1) if j else v for j, v in enumerate(pr)]
            z_rows.append(jnp.concatenate(barrel(rolled + [None] * 3, [(-i) % 8 for i in range(8)]), axis=1))
        return jnp.concatenate(p_rows, axis=0), jnp.concatenate(z_rows, axis=0)

    load_group(0)
    load_group(1)
    pre(0)
    for t in range(4):
        o_s[t, 0:128, :] = jnp.zeros((128, 128), F32)

    def out_copy(g):
        return pltpu.make_async_copy(st_s.at[g, pl.ds(0, D)], out_hbm.at[:, slab(g * 128)], osem.at[0])

    def step(g, part, carry):
        s = 4 * g + part
        mem, attn, best, arg = carry
        hh = jnp.concatenate([parked(), mem], axis=0)
        h1 = hh[:, 0:384]

        tails = []
        for j in range(L // 8):
            v = hh[8 * j:8 * j + 8, 384:512]
            tails.append(jnp.concatenate([jnp.where(low, v, 0.0), jnp.where(low, 0.0, v)], axis=0))
        tails += [jnp.zeros((16, 128), F32)] * 3
        tail_rhs = [jnp.concatenate([tails[(b - i) % 8] for b in range(8)], axis=0).astype(BF16)
                    for i in range(8)]

        sc = [None] * (L // 8)
        kp = {t: [] for t in range(4)}
        vt = {t: [] for t in range(4)}
        kd, vd, tl, ul = {}, {}, {}, {}
        for op in ORDER:
            if op[0] == 'Q':
                q2 = jnp.dot(hh, pltpu.bitcast(wq2_s[...], BF16), preferred_element_type=F32)
            elif op[0] == 'K':
                t, n = int(op[1]), int(op[2:])
                h0 = kd.get(t, 0)
                kp[t].append(project(h1, wk1_s, t, h0, h0 + n))
                kd[t] = h0 + n
            elif op[0] == 'V':
                t, n = int(op[1]), int(op[2:])
                h0 = vd.get(t, 0)
                vt[t].append(project(h1, wv1_s, t, h0, h0 + n))
                vd[t] = h0 + n
            elif op[0] == 'T':
                i = int(op[1])
                tl[i] = lax.dot_general(q2[:, 128 * i:128 * i + 128], tail_rhs[i], NT, preferred_element_type=F32)
            elif op[0] == 'S':
                t, j = int(op[1]), int(op[2])
                kt = jnp.concatenate([piece[j] for piece in kp[t]], axis=0)
                r0 = 8 * j if j < SEG // 8 else 0
                d = lax.dot_general(hh[r0:, 128 * t:128 * t + 128], kt.astype(BF16), NT, preferred_element_type=F32)
                sc[j] = d if sc[j] is None else sc[j] + d
            elif op[0] == 'A':
                best, arg = post(jnp.maximum(s - 1, 0), attn, s > 0, best, arg)
            elif op[0] == 'B':
                pre(jnp.minimum(s + 1, NSEG - 1))
            elif op[0] == 'C':
                store_group(jnp.maximum(g - 2, 0), (part,))
            elif op[0] == 'D':
                load_group(jnp.minimum(g + 2, NG - 1), (part,))
            elif op[0] == 'X':
                p, z = softmax(sc, [tl[i] for i in range(8)])
            elif op[0] == 'U':
                i = int(op[1])
                ul[i] = jnp.dot(z[:, 128 * i:128 * i + 128], tail_rhs[i], preferred_element_type=F32)
        u = jnp.concatenate([ul[i] for i in range(8)], axis=1)
        vmat = jnp.concatenate(
            [jnp.concatenate([piece[j] for j in range(L // 8) for piece in vt[t]], axis=0) for t in range(4)],
            axis=1)
        o = jnp.dot(p, vmat.astype(BF16), preferred_element_type=F32)
        o3 = o[:, 384:512]
        o = jnp.concatenate([o[:, 0:384], o3 + pltpu.roll(o3, 64, 1)], axis=1)
        o = jnp.dot(u, pltpu.bitcast(wb2_s[...], BF16), preferred_element_type=F32) + o
        return o[0:M], o[M:L], best, arg

    def group(g, carry):
        for i in range(4):
            carry = step(g, i, carry)

        @pl.when(g == 0)
        def _():
            for cp in cp_x:
                cp.wait()

        @pl.when(g >= 2)
        def _():
            out_copy(g - 2).start()

        return carry

    init = (_dup(mem0_ref[...].astype(F32)), jnp.zeros((SEG, DP), F32),
            jnp.full((8, 128), -jnp.inf, F32), jnp.zeros((8, 128), jnp.int32))
    _, attn, best, arg = lax.fori_loop(0, NG, group, init)
    for cp in cp_ffn:
        cp.wait()
    best, arg = post(NSEG - 1, attn, True, best, arg)

    top = jnp.max(best, axis=0, keepdims=True)
    idx = jnp.min(jnp.where(best == top, arg, S - 1))
    idx = jnp.clip(idx, 0, S - 1)
    xsel = jnp.concatenate([h2_s[t, pl.ds(idx, 1), :] for t in range(4)], axis=1)
    xsel = jnp.broadcast_to(xsel, (8, DP))[:, 0:D]
    store_group(NG - 2)
    store_group(NG - 1)
    gate = jnp.dot(xsel, wg_v[...], preferred_element_type=F32)
    up = jnp.dot(xsel, wu_v[...], preferred_element_type=F32)
    for g in range(NG - 2, NG):
        out_copy(g).start()
    act = gate * jax.nn.sigmoid(gate) * up
    y = lax.dot_general(act, wd_v[...], NT, preferred_element_type=F32)
    y = _dup(y) * jax.nn.sigmoid(top[:, 0:1]) * vec_s[5]
    for t in range(4):
        o_s[t, pl.ds(idx, 1), :] = o_s[t, pl.ds(idx, 1), :] + y[0:1, 128 * t:128 * t + 128]
    for g in range(NG):
        out_copy(g).wait()
    store_group(idx // 128)
    patch = out_copy(idx // 128)
    patch.start()
    patch.wait()


@functools.partial(jax.jit, static_argnames=("A_seg_len",))
def pallas_adaLN_cond__memory_aug_recurrent_mem_tr__moe_arch_mod__prompt_kernel(
        A_x, A_mem0, A_Wq, A_Wk, A_Wv, A_Wo, A_seg_len, B_x, B_w_r, B_w_gate, B_w_up, B_w_down, c, w_mod):
    del B_x
    assert A_seg_len == SEG and A_x.shape == (1, S, D) and A_Wq.shape == (D, H, E)
    hbm = pl.BlockSpec(memory_space=pl.ANY)
    outT = pl.pallas_call(
        _kernel,
        out_shape=jax.ShapeDtypeStruct((D, S), A_x.dtype),
        in_specs=[hbm] * 12,
        out_specs=hbm,
        scratch_shapes=[
            pltpu.VMEM((M, D), BF16),
            pltpu.VMEM((D,), BF16),
            pltpu.VMEM((1, D), BF16),
            pltpu.VMEM((2, D * H, 128), BF16),
            pltpu.VMEM((2, D * H, 128), BF16),
            pltpu.VMEM((2, D * H, 128), BF16),
            pltpu.VMEM((2, H, D, 128), BF16),
            pltpu.VMEM((H, 3, D, 128), F32),
            pltpu.VMEM((H // 2, 128, DP), F32),
            pltpu.VMEM((D, 6 * D), BF16),
            pltpu.VMEM((D, FF), BF16),
            pltpu.VMEM((D, FF), BF16),
            pltpu.VMEM((D, FF), BF16),
            pltpu.VMEM((NG, DP, 128), BF16),
            pltpu.VMEM((192, NW), U32),
            pltpu.VMEM((DP // 2, 64 * H), U32),
            pltpu.VMEM((192, NW), U32),
            pltpu.VMEM((32 * H, DP), U32),
            pltpu.VMEM((7, 8, DP), F32),
            pltpu.VMEM((4, S, 128), F32),
            pltpu.VMEM((4, S + SEG, 128), F32),
            pltpu.VMEM((4, S + SEG, 128), F32),
            pltpu.VMEM((NG, DP, 128), BF16),
            pltpu.SemaphoreType.DMA((NSEM,)),
            pltpu.SemaphoreType.DMA((1,)),
        ],
        compiler_params=pltpu.CompilerParams(vmem_limit_bytes=100 * 1024 * 1024),
        name="adaln_rmt_mod",
    )(
        A_x.reshape(S, D).T,
        A_mem0.reshape(M, D),
        A_Wq.reshape(D * H, E),
        A_Wk.reshape(D * H, E),
        A_Wv.reshape(D * H, E),
        A_Wo.transpose(0, 2, 1),
        B_w_r,
        B_w_gate,
        B_w_up,
        B_w_down.T,
        c,
        w_mod,
    )
    return outT.T.reshape(1, S, D)
```
